```python
import jax
import jax.numpy as jnp

def _softmax(x, axis=-1):
    return jax.nn.softmax(x, axis=axis)

def _gelu(x):
    return jax.nn.gelu(x, approximate=True)

def _silu(x):
    return jax.nn.silu(x)

def _sigmoid(x):
    return jax.nn.sigmoid(x)

def _layernorm(x, axis=-1, eps=1e-05):
    m = jnp.mean(x, axis=axis, keepdims=True)
    v = jnp.var(x, axis=axis, keepdims=True)
    return (x - m) / jnp.sqrt(v + eps)

def _scatter_add(tgt, idx, src, axis=0):
    return tgt.at[idx].add(src)

def _segment_sum(src, seg, n):
    return jax.ops.segment_sum(src, seg, n)

class _Rng:

    def __init__(self, key):
        self._k = key

    def _next(self):
        self._k, sub = jax.random.split(self._k)
        return sub

    def normal(self, shape):
        return jax.random.normal(self._next(), shape, dtype=jnp.bfloat16)

    def randint(self, lo, hi, shape):
        return jax.random.randint(self._next(), shape, lo, hi, dtype=jnp.int32)

    def uniform(self, shape, lo=0.0, hi=1.0):
        return jax.random.uniform(self._next(), shape, jnp.bfloat16, lo, hi)

    def permutation(self, n):
        return jax.random.permutation(self._next(), n)
kernel_name = 'interleave_layers__memory_aug_recurrent_mem_tr__sliding_local_dilated__prompt'

def setup_inputs():
    _rng = _Rng(jax.random.key(int.from_bytes(__import__("os").urandom(4), "little")))
    _w = lambda a: (lambda t: t.astype(jnp.bfloat16) if jnp.issubdtype(t.dtype, jnp.floating) else t)(jnp.asarray(a))

    def _A_setup():
        B, S, Dm = (1, 2048, 640)
        H, Dh = (32, 192)
        M, seg = (8, 32)
        seg = min(seg, S)
        S = S // seg * seg
        return {'x': _w((lambda *s: _rng.normal(s) * 0.05)(B, S, Dm)), 'mem0': _w((lambda *s: _rng.normal(s) * 0.05)(B, M, Dm)), 'Wq': _w((lambda *s: _rng.normal(s) * 0.05)(Dm, H, Dh) * Dm ** (-0.5)), 'Wk': _w((lambda *s: _rng.normal(s) * 0.05)(Dm, H, Dh) * Dm ** (-0.5)), 'Wv': _w((lambda *s: _rng.normal(s) * 0.05)(Dm, H, Dh) * Dm ** (-0.5)), 'Wo': _w((lambda *s: _rng.normal(s) * 0.05)(H, Dh, Dm) * (H * Dh) ** (-0.5)), 'seg_len': seg}
    _A_in = _A_setup()

    def _B_setup():
        B, S, D = (1, 2048, 640)
        return {'x': _w((lambda *s: _rng.normal(s) * 0.05)(B, S, D)), 'wqkv': _w((lambda *s: _rng.normal(s) * 0.05)(D, 3 * D)), 'wo': _w((lambda *s: _rng.normal(s) * 0.05)(D, D))}
    _B_in = _B_setup()
    return {'A_x': _A_in['x'], 'A_mem0': _A_in['mem0'], 'A_Wq': _A_in['Wq'], 'A_Wk': _A_in['Wk'], 'A_Wv': _A_in['Wv'], 'A_Wo': _A_in['Wo'], 'A_seg_len': _A_in['seg_len'], 'B_x': _B_in['x'], 'B_wqkv': _B_in['wqkv'], 'B_wo': _B_in['wo']}

def reference(A_x, A_mem0, A_Wq, A_Wk, A_Wv, A_Wo, A_seg_len, B_x, B_wqkv, B_wo):

    def _A_ref(x, mem0, Wq, Wk, Wv, Wo, seg_len):
        B, S, Dm = x.shape
        H, Dh = (Wq.shape[1], Wq.shape[2])
        M = mem0.shape[1]
        scale = Dh ** (-0.5)
        n_seg = S // seg_len
        L = M + seg_len
        idx = jnp.arange(L)
        mask = (idx[:, None] < M) | (idx[:, None] >= idx[None, :])
        mem = mem0
        outs = []
        for s in range(n_seg):
            xs = x[:, s * seg_len:(s + 1) * seg_len, :].copy()
            h = jnp.concatenate([mem, xs], axis=1)
            q = jnp.einsum('btd,dhe->bhte', h, Wq)
            k = jnp.einsum('btd,dhe->bhte', h, Wk)
            v = jnp.einsum('btd,dhe->bhte', h, Wv)
            scores = jnp.einsum('bhqe,bhke->bhqk', q, k) * scale
            scores = jnp.where(mask[None, None], scores, -1000000000.0)
            p = _softmax(scores, axis=-1)
            o = jnp.einsum('bhqk,bhke->bhqe', p, v)
            o = jnp.einsum('bhte,hed->btd', o, Wo)
            mem = o[:, :M, :].copy()
            outs.append(o[:, M:, :])
        return jnp.concatenate(outs, axis=1)

    def _B_ref(x, wqkv, wo):
        B, S, D = x.shape
        H = 32
        Dh = D // H
        W, dil = (8, 2)
        qkv = (lambda x, *d: x.transpose(*d))((x @ wqkv).reshape(B, S, 3, H, Dh), 2, 0, 3, 1, 4)
        q, k, v = (qkv[0], qkv[1], qkv[2])
        scale = Dh ** (-0.5)
        pos = jnp.arange(S)
        off = jnp.arange(W) * dil
        idx = pos[:, None] - off[None, :]
        mask = idx >= 0
        idx_c = jnp.where(mask, idx, 0).reshape(-1)
        kg = k[:, :, idx_c, :].reshape(B, H, S, W, Dh)
        vg = v[:, :, idx_c, :].reshape(B, H, S, W, Dh)
        logits = jnp.einsum('bhsd,bhswd->bhsw', q, kg) * scale
        logits = jnp.where(mask[None, None, :, :], logits, -1000000000.0)
        attn = _softmax(logits, axis=-1)
        o = jnp.einsum('bhsw,bhswd->bhsd', attn, vg)
        return (lambda x, *d: x.transpose(*d))(o, 0, 2, 1, 3).reshape(B, S, D) @ wo
    x = A_x
    x = x + _A_ref(_layernorm(x, axis=-1), A_mem0, A_Wq, A_Wk, A_Wv, A_Wo, A_seg_len)
    x = x + _B_ref(_layernorm(x, axis=-1), B_wqkv, B_wo)
    x = x + _A_ref(_layernorm(x, axis=-1), A_mem0, A_Wq, A_Wk, A_Wv, A_Wo, A_seg_len)
    x = x + _B_ref(_layernorm(x, axis=-1), B_wqkv, B_wo)
    return x
```

```python
import functools
import numpy as np
import jax
import jax.numpy as jnp
from jax import lax
import jax.experimental.pallas as pl
import jax.experimental.pallas.tpu as pltpu

F32 = jnp.float32
BF16 = jnp.bfloat16


def _ln(x):
    m = jnp.mean(x, axis=-1, keepdims=True)
    xc = x - m
    v = jnp.mean(xc * xc, axis=-1, keepdims=True)
    return xc * lax.rsqrt(v + 1e-5)


def _dot(a, b):
    return jnp.dot(a, b, preferred_element_type=F32)


def _dot_nt(a, b):
    return lax.dot_general(a, b, (((1,), (1,)), ((), ())), preferred_element_type=F32)


def _kernel(x_ref, mem0_ref, wq_ref, wk_ref, wv_ref, wo_ref, bqkv_ref, bwo_ref, o_ref,
            xb_scr, x2_scr, mem_scr, kprev_scr, vprev_scr, *, nseg):
    SEG, M, D = 32, 8, 640
    L = M + SEG
    scale_a = 192 ** -0.5
    scale_b = 20 ** -0.5

    xb_scr[...] = jnp.zeros_like(xb_scr)
    x2_scr[...] = jnp.zeros_like(x2_scr)
    kprev_scr[...] = jnp.zeros_like(kprev_scr)
    vprev_scr[...] = jnp.zeros_like(vprev_scr)
    mem0 = mem0_ref[...].astype(F32)
    mem_scr[0:8, :] = mem0
    mem_scr[8:16, :] = mem0

    r = lax.broadcasted_iota(jnp.int32, (2 * L, 2 * L), 0)
    c = lax.broadcasted_iota(jnp.int32, (2 * L, 2 * L), 1)
    rl = jnp.where(r >= L, 1, 0)
    cl = jnp.where(c >= L, 1, 0)
    rr = r - rl * L
    cc = c - cl * L
    amask = (rl == cl) & ((rr < M) | (rr >= cc))
    lane = lax.broadcasted_iota(jnp.int32, (2 * L, 128), 1)
    lo = lane < 64

    def b_phase(t):
        xb = xb_scr[...]
        hb = _ln(xb).astype(BF16)
        qkv = _dot(hb, bqkv_ref[...])
        row = lax.broadcasted_iota(jnp.int32, (SEG, 128), 0)
        outs = []
        for l in range(2):
            seg = t - 1 - 2 * l
            q = qkv[l * SEG:(l + 1) * SEG, 0:D]
            k = qkv[l * SEG:(l + 1) * SEG, D:2 * D]
            v = qkv[l * SEG:(l + 1) * SEG, 2 * D:3 * D]
            kk = jnp.concatenate([kprev_scr[l], k], axis=0)
            vv = jnp.concatenate([vprev_scr[l], v], axis=0)
            kprev_scr[l] = k[16:32]
            vprev_scr[l] = v[16:32]
            logits = []
            for w in range(8):
                ks = kk[16 - 2 * w:48 - 2 * w]
                y = q[:, 0:128] * ks[:, 0:128]
                for tau in range(1, 5):
                    y = y + q[:, tau * 128:(tau + 1) * 128] * ks[:, tau * 128:(tau + 1) * 128]
                y = y + pltpu.roll(y, 64, 1)
                y = y + pltpu.roll(y, 32, 1)
                valid = (seg * SEG + row - 2 * w) >= 0
                logits.append(jnp.where(valid, y * scale_b, -1e9))
            mx = logits[0]
            for w in range(1, 8):
                mx = jnp.maximum(mx, logits[w])
            es = [jnp.exp(lg - mx) for lg in logits]
            sm = es[0]
            for w in range(1, 8):
                sm = sm + es[w]
            inv = 1.0 / sm
            o_t = [None] * 5
            for w in range(8):
                p = es[w] * inv
                vs = vv[16 - 2 * w:48 - 2 * w]
                for tau in range(5):
                    term = p * vs[:, tau * 128:(tau + 1) * 128]
                    o_t[tau] = term if o_t[tau] is None else o_t[tau] + term
            outs.append(jnp.concatenate(o_t, axis=1))
        ob = jnp.concatenate(outs, axis=0).astype(BF16)
        return xb + _dot(ob, bwo_ref[...])

    def step(t, _):
        xo = b_phase(t)
        xa2 = x2_scr[...]
        x2_scr[...] = xo[0:SEG]
        so = jnp.maximum(t - 3, 0)
        o_ref[pl.ds(pl.multiple_of(so * SEG, SEG), SEG), :] = xo[SEG:2 * SEG].astype(o_ref.dtype)

        sa = jnp.minimum(t, nseg - 1)
        xa1 = x_ref[pl.ds(pl.multiple_of(sa * SEG, SEG), SEG), :].astype(F32)
        mem1 = mem_scr[0:8, :]
        mem2 = jnp.where(t <= 2, mem0, mem_scr[8:16, :])
        h = jnp.concatenate([mem1, _ln(xa1), mem2, _ln(xa2)], axis=0).astype(BF16)
        acc = None
        for j in range(16):
            c0 = j * 384
            q = _dot(h, wq_ref[:, c0:c0 + 384]).astype(BF16)
            k = _dot(h, wk_ref[:, c0:c0 + 384]).astype(BF16)
            v = _dot(h, wv_ref[:, c0:c0 + 384]).astype(BF16)
            q0, qm, q2 = q[:, 0:128], q[:, 128:256], q[:, 256:384]
            k0, km, k2 = k[:, 0:128], k[:, 128:256], k[:, 256:384]
            v0, vm, v2 = v[:, 0:128], v[:, 128:256], v[:, 256:384]
            zero = jnp.zeros_like(qm)
            s0 = _dot_nt(q0, k0) + _dot_nt(jnp.where(lo, qm, zero), km)
            s1 = _dot_nt(jnp.where(lo, zero, qm), km) + _dot_nt(q2, k2)
            ps = []
            for s in (s0, s1):
                s = jnp.where(amask, s * scale_a, -1e9)
                mx = jnp.max(s, axis=1, keepdims=True)
                e = jnp.exp(s - mx)
                p = e / jnp.sum(e, axis=1, keepdims=True)
                ps.append(p.astype(BF16))
            o0 = _dot(ps[0], v0)
            om = jnp.where(lo, _dot(ps[0], vm), _dot(ps[1], vm))
            o2 = _dot(ps[1], v2)
            o = jnp.concatenate([o0, om, o2], axis=1).astype(BF16)
            contrib = _dot(o, wo_ref[c0:c0 + 384, :])
            acc = contrib if acc is None else acc + contrib
        mem_scr[0:8, :] = acc[0:8]
        mem_scr[8:16, :] = acc[L:L + 8]
        xb_scr[0:SEG, :] = xa1 + acc[8:L]
        xb_scr[SEG:2 * SEG, :] = xa2 + acc[L + 8:2 * L]
        return 0

    lax.fori_loop(0, nseg + 2, step, 0)
    xo = b_phase(nseg + 2)
    o_ref[pl.ds((nseg - 1) * SEG, SEG), :] = xo[SEG:2 * SEG].astype(o_ref.dtype)


@functools.partial(jax.jit, static_argnames=("A_seg_len",))
def pallas_interleave_layers__memory_aug_recurrent_mem_tr__sliding_local_dilated__prompt_kernel(
        A_x, A_mem0, A_Wq, A_Wk, A_Wv, A_Wo, A_seg_len, B_x, B_wqkv, B_wo):
    S, D = A_x.shape[1], A_x.shape[2]
    x = A_x.reshape(S, D)
    mem0 = A_mem0.reshape(8, D)
    wq = A_Wq.reshape(D, 6144)
    wk = A_Wk.reshape(D, 6144)
    wv = A_Wv.reshape(D, 6144)
    wo = A_Wo.reshape(6144, D)
    bqkv = B_wqkv.reshape(D, 3, 32, 20).transpose(0, 1, 3, 2).reshape(D, 3 * D)
    bwo = B_wo.reshape(32, 20, D).transpose(1, 0, 2).reshape(D, D)
    out = pl.pallas_call(
        functools.partial(_kernel, nseg=S // 32),
        out_shape=jax.ShapeDtypeStruct((S, D), A_x.dtype),
        scratch_shapes=[
            pltpu.VMEM((64, D), F32),
            pltpu.VMEM((32, D), F32),
            pltpu.VMEM((16, D), F32),
            pltpu.VMEM((2, 16, D), F32),
            pltpu.VMEM((2, 16, D), F32),
        ],
        compiler_params=pltpu.CompilerParams(vmem_limit_bytes=100 * 1024 * 1024),
    )(x, mem0, wq, wk, wv, wo, bqkv, bwo)
    return out.reshape(A_x.shape)
```

```python
import functools
import numpy as np
import jax
import jax.numpy as jnp
from jax import lax
import jax.experimental.pallas as pl
import jax.experimental.pallas.tpu as pltpu

F32 = jnp.float32
BF16 = jnp.bfloat16
ATT = "comb"
SINGLE = "1" == "1"
TAIL = "1" == "1"

SEG, M, D = 32, 8, 640
L = M + SEG
NP = 16
PW = 384
NEG = -1e9


def _ln(x):
    m = jnp.mean(x, axis=-1, keepdims=True)
    xc = x - m
    v = jnp.mean(xc * xc, axis=-1, keepdims=True)
    return xc * lax.rsqrt(v + 1e-5)


def _dot(a, b):
    return jnp.dot(a, b, preferred_element_type=F32)


def _dot_nt(a, b):
    return lax.dot_general(a, b, (((1,), (1,)), ((), ())), preferred_element_type=F32)


def _iota(shape, dim):
    return lax.broadcasted_iota(jnp.int32, shape, dim)


def _kernel(x_hbm, mem0_hbm, wq_hbm, wk_hbm, wv_hbm, wo_hbm, bqkv_hbm, bwo_hbm, o_hbm,
            wq_ref, wk_ref, wv_ref, wo_ref, braw_ref, bworaw_ref, bqkv_ref, bwo_ref, x_ref, o_ref, mem0_ref,
            xb_scr, x2_scr, mem_scr, kprev_scr, vprev_scr, wsem, msem, *, nseg):
    scale_a = 192 ** -0.5
    scale_b = 20 ** -0.5

    def wcopies(j):
        sl = pl.ds(j * PW, PW)
        return [pltpu.make_async_copy(src.at[sl, :], dst.at[sl, :], wsem.at[j])
                for src, dst in ((wq_hbm, wq_ref), (wk_hbm, wk_ref), (wv_hbm, wv_ref), (wo_hbm, wo_ref))]

    def misc_copies():
        return [pltpu.make_async_copy(bqkv_hbm, braw_ref, msem.at[0]),
                pltpu.make_async_copy(bwo_hbm, bworaw_ref, msem.at[1]),
                pltpu.make_async_copy(x_hbm, x_ref, msem.at[2]),
                pltpu.make_async_copy(mem0_hbm, mem0_ref, msem.at[3])]

    LOOK = 3
    mc = misc_copies()
    mc[2].start()
    mc[3].start()
    for c in wcopies(0):
        c.start()
    mc[0].start()
    mc[1].start()
    for j in range(1, LOOK):
        for c in wcopies(j):
            c.start()

    xb_scr[...] = jnp.zeros_like(xb_scr)
    x2_scr[...] = jnp.zeros_like(x2_scr)
    kprev_scr[...] = jnp.zeros_like(kprev_scr)
    vprev_scr[...] = jnp.zeros_like(vprev_scr)
    mc[2].wait()
    mc[3].wait()
    mem0 = mem0_ref[...].astype(F32)
    mem_scr[0:8, :] = mem0
    mem_scr[8:16, :] = mem0

    def permute_b_weights():
        mc[0].wait()
        mc[1].wait()
        for nt in range(5):
            n = _iota((D, 128), 1) + nt * 128
            i = _iota((D, 128), 0)
            src = (n & 31) * 20 + (n >> 5)
            pm = jnp.where(i == src, 1.0, 0.0).astype(BF16)
            for part in range(3):
                w = braw_ref[:, part * D:(part + 1) * D]
                bqkv_ref[:, part * D + nt * 128:part * D + (nt + 1) * 128] = _dot(w, pm).astype(BF16)
        for nt in range(5):
            n = _iota((128, D), 0) + nt * 128
            i = _iota((128, D), 1)
            src = (n & 31) * 20 + (n >> 5)
            pmt = jnp.where(i == src, 1.0, 0.0).astype(BF16)
            bwo_ref[nt * 128:(nt + 1) * 128, :] = _dot(pmt, bworaw_ref[...]).astype(BF16)

    def att_masks(rows):
        r = _iota((rows, 2 * L), 0)
        c = _iota((rows, 2 * L), 1)
        rl = jnp.where(r >= L, 1, 0)
        cl = jnp.where(c >= L, 1, 0)
        rr = r - rl * L
        cc = c - cl * L
        causal = (rr < M) | (rr >= cc)
        return rl, cl, causal

    def b_qkv():
        xb = xb_scr[...]
        hb = _ln(xb).astype(BF16)
        qkv = _dot(hb, bqkv_ref[...])
        return xb, qkv

    def b_attn(t, qkv):
        row = _iota((SEG, 128), 0)
        outs = []
        for l in range(2):
            seg = t - 1 - 2 * l
            q = qkv[l * SEG:(l + 1) * SEG, 0:D]
            k = qkv[l * SEG:(l + 1) * SEG, D:2 * D]
            v = qkv[l * SEG:(l + 1) * SEG, 2 * D:3 * D]
            kk = jnp.concatenate([kprev_scr[l], k], axis=0)
            vv = jnp.concatenate([vprev_scr[l], v], axis=0)
            kprev_scr[l] = k[16:32]
            vprev_scr[l] = v[16:32]
            logits = []
            for w in range(8):
                ks = kk[16 - 2 * w:48 - 2 * w]
                y = q[:, 0:128] * ks[:, 0:128]
                for tau in range(1, 5):
                    y = y + q[:, tau * 128:(tau + 1) * 128] * ks[:, tau * 128:(tau + 1) * 128]
                y = y + pltpu.roll(y, 64, 1)
                y = y + pltpu.roll(y, 32, 1)
                valid = (seg * SEG + row - 2 * w) >= 0
                logits.append(jnp.where(valid, y * scale_b, NEG))
            mx = logits[0]
            for w in range(1, 8):
                mx = jnp.maximum(mx, logits[w])
            es = [jnp.exp(lg - mx) for lg in logits]
            sm = es[0]
            for w in range(1, 8):
                sm = sm + es[w]
            inv = 1.0 / sm
            o_t = [None] * 5
            for w in range(8):
                p = es[w] * inv
                vs = vv[16 - 2 * w:48 - 2 * w]
                for tau in range(5):
                    term = p * vs[:, tau * 128:(tau + 1) * 128]
                    o_t[tau] = term if o_t[tau] is None else o_t[tau] + term
            outs.append(jnp.concatenate(o_t, axis=1))
        return jnp.concatenate(outs, axis=0).astype(BF16)

    def b_out_cols(xb, ob, c0, c1):
        return xb[:, c0:c1] + _dot(ob, bwo_ref[:, c0:c1])

    def proj(h, w_ref, j):
        return _dot_nt(h, w_ref[j * PW:(j + 1) * PW, :])

    def t3(a):
        return a[:, 0:128], a[:, 128:256], a[:, 256:384]

    def softmax_comb(s, causal, left):
        s = jnp.where(causal, s * scale_a, NEG)
        m_lo = jnp.max(jnp.where(left, s, NEG), axis=1, keepdims=True)
        m_hi = jnp.max(jnp.where(left, NEG, s), axis=1, keepdims=True)
        e = jnp.exp(s - jnp.where(left, m_lo, m_hi))
        s_lo = jnp.sum(jnp.where(left, e, 0.0), axis=1, keepdims=True)
        s_hi = jnp.sum(jnp.where(left, 0.0, e), axis=1, keepdims=True)
        return e * jnp.where(left, 1.0 / s_lo, 1.0 / s_hi)

    def make_att(rows):
        lane = _iota((L, 128), 1)
        lo = lane < 64
        rl, cl, causal = att_masks(rows)
        left = cl == 0
        diag = rl == cl
        zero40 = jnp.zeros((L, 128), F32)

        def split_mid(a, swap):
            x0 = jnp.where(lo, a, 0.0)
            x1 = jnp.where(lo, 0.0, a)
            return jnp.concatenate([x1, x0] if swap else [x0, x1], axis=0).astype(BF16)

        if rows == L:
            def scores(q, k):
                q0, qm, q2 = t3(q)
                k0, km, k2 = t3(k)
                r0 = jnp.concatenate([k0, zero40], axis=0).astype(BF16)
                r2 = jnp.concatenate([zero40, k2], axis=0).astype(BF16)
                return _dot_nt(q0, r0) + _dot_nt(q2, r2) + _dot_nt(qm, split_mid(km, False))

            def smax(s):
                return softmax_comb(s, causal, left)

            def pv(p, v):
                v0, vm, v2 = t3(v)
                r0 = jnp.concatenate([v0, zero40], axis=0).astype(BF16)
                r2 = jnp.concatenate([zero40, v2], axis=0).astype(BF16)
                return jnp.concatenate([_dot(p, r0), _dot(p, split_mid(vm, False)), _dot(p, r2)], axis=1)
        elif ATT == "comb":
            def scores(q, k):
                q0, qm, q2 = t3(q)
                k0, km, k2 = t3(k)
                k2s = jnp.concatenate([k2[L:2 * L], k2[0:L]], axis=0)
                s0 = _dot_nt(q0, k0.astype(BF16))
                s2 = _dot_nt(q2, k2s.astype(BF16))
                mid = jnp.concatenate([_dot_nt(qm[0:L], split_mid(km[0:L], False)),
                                       _dot_nt(qm[L:2 * L], split_mid(km[L:2 * L], True))], axis=0)
                return jnp.where(diag, s0, s2) + mid

            def smax(s):
                return softmax_comb(s, causal, left)

            def pv(p, v):
                v0, vm, v2 = t3(v)
                v2s = jnp.concatenate([v2[L:2 * L], v2[0:L]], axis=0)
                p0 = jnp.where(diag, p, 0.0)
                p1 = jnp.where(diag, 0.0, p)
                o0 = _dot(p0, v0.astype(BF16))
                o2 = _dot(p1, v2s.astype(BF16))
                om = jnp.concatenate([_dot(p[0:L], split_mid(vm[0:L], False)),
                                      _dot(p[L:2 * L], split_mid(vm[L:2 * L], True))], axis=0)
                return jnp.concatenate([o0, om, o2], axis=1)
        else:
            lo80 = _iota((2 * L, 128), 1) < 64
            amask = diag & causal

            def scores(q, k):
                q0, qm, q2 = t3(q)
                k0, km, k2 = t3(k.astype(BF16))
                s0 = _dot_nt(q0, k0) + _dot_nt(jnp.where(lo80, qm, 0.0), km)
                s1 = _dot_nt(jnp.where(lo80, 0.0, qm), km) + _dot_nt(q2, k2)
                return s0, s1

            def smax(ss):
                out = []
                for s in ss:
                    s = jnp.where(amask, s * scale_a, NEG)
                    mx = jnp.max(s, axis=1, keepdims=True)
                    e = jnp.exp(s - mx)
                    out.append(e * (1.0 / jnp.sum(e, axis=1, keepdims=True)))
                return out

            def pv(ps, v):
                p0, p1 = ps
                v0, vm, v2 = t3(v.astype(BF16))
                o0 = _dot(p0, v0)
                om = jnp.where(lo80, _dot(p0, vm), _dot(p1, vm))
                o2 = _dot(p1, v2)
                return jnp.concatenate([o0, om, o2], axis=1)
        return scores, smax, pv

    def a_pass(h, rows, first, pre_hook=None, mid_hook=None, tail_x=None, tail_y=None):
        scores, smax, pv = make_att(rows)

        def wait(j):
            if first:
                for c in wcopies(j):
                    c.wait()
                if j + LOOK < NP:
                    for c in wcopies(j + LOOK):
                        c.start()

        def outproj(o, j):
            return _dot(o, wo_ref[j * PW:(j + 1) * PW, :])

        wait(0)
        q = proj(h, wq_ref, 0)
        k = proj(h, wk_ref, 0)
        v = proj(h, wv_ref, 0)
        if pre_hook is not None:
            pre_hook()
        acc = None
        o_def = None
        for j in range(NP):
            s = scores(q, k)
            if j < NP - 1:
                wait(j + 1)
                qn = proj(h, wq_ref, j + 1)
                kn = proj(h, wk_ref, j + 1)
            else:
                if o_def is not None:
                    acc = acc + outproj(o_def, j - 1)
                if tail_x is not None:
                    tail_x()
            p = smax(s)
            if j == 8 and mid_hook is not None:
                mid_hook()
            o = pv(p, v)
            if j < NP - 1:
                vn = proj(h, wv_ref, j + 1)
            elif tail_y is not None:
                tail_y()
            if TAIL and j == NP - 2:
                o_def = o
            else:
                contrib = outproj(o, j)
                acc = contrib if acc is None else acc + contrib
            if j < NP - 1:
                q, k, v = qn, kn, vn
        return acc

    def xseg(s):
        return x_ref[pl.ds(pl.multiple_of(s * SEG, SEG), SEG), :].astype(F32)

    def store_out(s, val):
        o_ref[pl.ds(pl.multiple_of(s * SEG, SEG), SEG), :] = val.astype(o_ref.dtype)

    def step_double(t):
        st = {}
        xa2 = x2_scr[...]
        xa1 = xseg(jnp.minimum(t, nseg - 1))
        mem1 = mem_scr[0:8, :]
        mem2 = mem_scr[8:16, :]
        h = jnp.concatenate([mem1, _ln(xa1), mem2, _ln(xa2)], axis=0).astype(BF16)

        def pre():
            st['xb'], st['bq'] = b_qkv()

        def mid():
            st['ob'] = b_attn(t, st['bq'])

        def tx():
            st['xo0'] = b_out_cols(st['xb'], st['ob'], 0, 384)

        def ty():
            st['xo1'] = b_out_cols(st['xb'], st['ob'], 384, 640)
        acc = a_pass(h, 2 * L, False, pre, mid, tx, ty)
        xo = jnp.concatenate([st['xo0'], st['xo1']], axis=1)
        x2_scr[...] = xo[0:SEG]
        store_out(jnp.maximum(t - 3, 0), xo[SEG:2 * SEG])
        mem_scr[0:8, :] = acc[0:8]
        mem_scr[8:16, :] = acc[L:L + 8]
        xb_scr[0:SEG, :] = xa1 + acc[8:L]
        xb_scr[SEG:2 * SEG, :] = xa2 + acc[L + 8:2 * L]

    def step_single(t, layer, first):
        st = {}
        if layer == 0:
            xa = xseg(t)
        else:
            xa = x2_scr[...]
        mem = mem_scr[layer * 8:layer * 8 + 8, :]
        h = jnp.concatenate([mem, _ln(xa)], axis=0)
        if first:
            acc = a_pass(h, L, True)
        else:
            def pre():
                st['xb'], st['bq'] = b_qkv()

            def mid():
                st['ob'] = b_attn(t, st['bq'])

            def tx():
                st['xo0'] = b_out_cols(st['xb'], st['ob'], 0, 384)

            def ty():
                st['xo1'] = b_out_cols(st['xb'], st['ob'], 384, 640)
            acc = a_pass(h, L, False, pre, mid, tx, ty)
            xo = jnp.concatenate([st['xo0'], st['xo1']], axis=1)
            x2_scr[...] = xo[0:SEG]
            store_out(max(t - 3, 0), xo[SEG:2 * SEG])
        mem_scr[layer * 8:layer * 8 + 8, :] = acc[0:8]
        xb_scr[layer * SEG:(layer + 1) * SEG, :] = xa + acc[8:L]

    if SINGLE:
        step_single(0, 0, True)
        permute_b_weights()
        step_single(1, 0, False)

        def body(t, _):
            step_double(t)
            return 0
        lax.fori_loop(2, nseg, body, 0)
        step_single(nseg, 1, False)
        step_single(nseg + 1, 1, False)
    else:
        for j in range(NP):
            if j + LOOK < NP:
                for c in wcopies(j + LOOK):
                    c.start()
        for j in range(NP):
            for c in wcopies(j):
                c.wait()
        permute_b_weights()

        def body(t, _):
            @pl.when(t == 2)
            def _():
                mem_scr[8:16, :] = mem0_ref[...].astype(F32)
            step_double(t)
            return 0
        lax.fori_loop(0, nseg + 2, body, 0)
    xb, bq = b_qkv()
    ob = b_attn(nseg + 2, bq)
    xo = b_out_cols(xb, ob, 0, D)
    store_out(nseg - 1, xo[SEG:2 * SEG])
    oc = pltpu.make_async_copy(o_ref, o_hbm, msem.at[0])
    oc.start()
    oc.wait()


@functools.partial(jax.jit, static_argnames=("A_seg_len",))
def pallas_interleave_layers__memory_aug_recurrent_mem_tr__sliding_local_dilated__prompt_kernel(
        A_x, A_mem0, A_Wq, A_Wk, A_Wv, A_Wo, A_seg_len, B_x, B_wqkv, B_wo):
    S = A_x.shape[1]
    x = A_x.reshape(S, D)
    mem0 = A_mem0.reshape(8, D)
    wq = A_Wq.transpose(1, 2, 0).reshape(6144, D)
    wk = A_Wk.transpose(1, 2, 0).reshape(6144, D)
    wv = A_Wv.transpose(1, 2, 0).reshape(6144, D)
    wo = A_Wo.reshape(6144, D)
    anyspec = pl.BlockSpec(memory_space=pl.ANY)
    out = pl.pallas_call(
        functools.partial(_kernel, nseg=S // 32),
        out_shape=jax.ShapeDtypeStruct((S, D), A_x.dtype),
        in_specs=[anyspec] * 8,
        out_specs=anyspec,
        scratch_shapes=[
            pltpu.VMEM((6144, D), BF16), pltpu.VMEM((6144, D), BF16), pltpu.VMEM((6144, D), BF16), pltpu.VMEM((6144, D), BF16),
            pltpu.VMEM((D, 3 * D), BF16), pltpu.VMEM((D, D), BF16),
            pltpu.VMEM((D, 3 * D), BF16), pltpu.VMEM((D, D), BF16),
            pltpu.VMEM((S, D), BF16), pltpu.VMEM((S, D), BF16), pltpu.VMEM((8, D), BF16),
            pltpu.VMEM((64, D), F32),
            pltpu.VMEM((32, D), F32),
            pltpu.VMEM((16, D), F32),
            pltpu.VMEM((2, 16, D), F32),
            pltpu.VMEM((2, 16, D), F32),
            pltpu.SemaphoreType.DMA((NP,)),
            pltpu.SemaphoreType.DMA((4,)),
        ],
        compiler_params=pltpu.CompilerParams(vmem_limit_bytes=100 * 1024 * 1024),
    )(x, mem0, wq, wk, wv, wo, B_wqkv, B_wo)
    return out.reshape(A_x.shape)
```

```python
import functools
import numpy as np
import jax
import jax.numpy as jnp
from jax import lax
import jax.experimental.pallas as pl
import jax.experimental.pallas.tpu as pltpu

F32 = jnp.float32
BF16 = jnp.bfloat16

SEG, M, D = 32, 8, 640
L = M + SEG
NP = 16
PW = 384
NEG = -1e9
RN = 16
PROWS = 288
R0 = 240
NPRE = (R0 + RN - SEG) // (SEG - RN) + 1
LOOK = 5
PSCHED = [0, 0, 0, 0, 0, 1, 2, 2, 3, 4]
assert R0 % RN == 0 and R0 + 2 * RN <= PROWS and PROWS % RN == 0 and PROWS % SEG == 0


def _ln(x):
    m = jnp.mean(x, axis=-1, keepdims=True)
    xc = x - m
    v = jnp.mean(xc * xc, axis=-1, keepdims=True)
    return xc * lax.rsqrt(v + 1e-5)


def _dot(a, b):
    return jnp.dot(a, b, preferred_element_type=F32)


def _dot_nt(a, b):
    return lax.dot_general(a, b, (((1,), (1,)), ((), ())), preferred_element_type=F32)


def _iota(shape, dim):
    return lax.broadcasted_iota(jnp.int32, shape, dim)


def _kernel(x_hbm, mem0_hbm, wq_hbm, wk_hbm, wv_hbm, wo_hbm, bqkv_hbm, bwo_hbm, o_hbm,
            w_ref, braw_ref, bworaw_ref, bqkv_ref, bwo_ref, x_ref, o_ref, mem0_ref,
            xb_scr, x2_scr, lx2_scr, mem_scr, kprev_scr, vprev_scr,
            pq_ref, pk_ref, pv_ref, lx_ref, wsem, msem, *, nseg):
    S_ROWS = nseg * SEG
    XH = 2 * SEG + R0 + SEG
    scale_a = 192 ** -0.5
    scale_b = 20 ** -0.5

    def wcopies(j):
        sl = pl.ds(j * PW, PW)
        return [pltpu.make_async_copy(hbm.at[sl, :], w_ref.at[j, i], wsem.at[j])
                for i, hbm in enumerate((wq_hbm, wk_hbm, wv_hbm, wo_hbm))]

    def start_pair(j):
        for c in wcopies(j):
            c.start()

    def wait_pair(j):
        pltpu.make_async_copy(w_ref.at[j], w_ref.at[j], wsem.at[j]).wait()

    cp_bqkv = pltpu.make_async_copy(bqkv_hbm, braw_ref, msem.at[0])
    cp_bwo = pltpu.make_async_copy(bwo_hbm, bworaw_ref, msem.at[1])
    cp_xh = pltpu.make_async_copy(x_hbm.at[pl.ds(0, XH), :], x_ref.at[pl.ds(0, XH), :], msem.at[2])
    cp_mem = pltpu.make_async_copy(mem0_hbm, mem0_ref, msem.at[3])
    cp_xr = pltpu.make_async_copy(x_hbm.at[pl.ds(XH, S_ROWS - XH), :], x_ref.at[pl.ds(XH, S_ROWS - XH), :], msem.at[4])

    cp_xh.start()
    cp_mem.start()
    cp_xh.wait()
    cp_mem.wait()
    cp_bwo.start()
    cp_bqkv.start()

    xb_scr[...] = jnp.zeros_like(xb_scr)
    x2_scr[...] = jnp.zeros_like(x2_scr)
    lx2_scr[...] = jnp.zeros_like(lx2_scr)
    kprev_scr[...] = jnp.zeros_like(kprev_scr)
    vprev_scr[...] = jnp.zeros_like(vprev_scr)
    lx_ref[0:XH, :] = _ln(x_ref[0:XH, :].astype(F32))
    mem0 = mem0_ref[...].astype(F32)
    mem_scr[0:8, :] = mem0
    mem_scr[8:16, :] = mem0

    def perm_qkv(nt):
        n = _iota((D, 128), 1) + nt * 128
        i = _iota((D, 128), 0)
        src = (n & 31) * 20 + (n >> 5)
        pm = jnp.where(i == src, 1.0, 0.0).astype(BF16)
        for part in range(3):
            w = braw_ref[:, part * D:(part + 1) * D]
            bqkv_ref[:, part * D + nt * 128:part * D + (nt + 1) * 128] = _dot(w, pm).astype(BF16)

    def perm_wo(nt):
        n = _iota((128, D), 0) + nt * 128
        i = _iota((128, D), 1)
        src = (n & 31) * 20 + (n >> 5)
        pmt = jnp.where(i == src, 1.0, 0.0).astype(BF16)
        bwo_ref[nt * 128:(nt + 1) * 128, :] = _dot(pmt, bworaw_ref[...]).astype(BF16)

    def perm_all():
        started = 0
        cp_bwo.wait()
        for i in range(10):
            while started < PSCHED[i]:
                start_pair(started)
                started += 1
            if i < 5:
                perm_wo(i)
            else:
                if i == 5:
                    cp_bqkv.wait()
                perm_qkv(i - 5)
        while started < LOOK:
            start_pair(started)
            started += 1

    def b_qkv():
        xb = xb_scr[...]
        hb = _ln(xb).astype(BF16)
        return xb, _dot(hb, bqkv_ref[...])

    def b_attn(t, qkv):
        row = _iota((SEG, 128), 0)
        outs = []
        for l in range(2):
            seg = t - 1 - 2 * l
            q = qkv[l * SEG:(l + 1) * SEG, 0:D]
            k = qkv[l * SEG:(l + 1) * SEG, D:2 * D]
            v = qkv[l * SEG:(l + 1) * SEG, 2 * D:3 * D]
            kk = jnp.concatenate([kprev_scr[l], k], axis=0)
            vv = jnp.concatenate([vprev_scr[l], v], axis=0)
            kprev_scr[l] = k[16:32]
            vprev_scr[l] = v[16:32]
            logits = []
            for w in range(8):
                ks = kk[16 - 2 * w:48 - 2 * w]
                y = q[:, 0:128] * ks[:, 0:128]
                for tau in range(1, 5):
                    y = y + q[:, tau * 128:(tau + 1) * 128] * ks[:, tau * 128:(tau + 1) * 128]
                y = y + pltpu.roll(y, 64, 1)
                y = y + pltpu.roll(y, 32, 1)
                valid = (seg * SEG + row - 2 * w) >= 0
                logits.append(jnp.where(valid, y * scale_b, NEG))
            mx = logits[0]
            for w in range(1, 8):
                mx = jnp.maximum(mx, logits[w])
            es = [jnp.exp(lg - mx) for lg in logits]
            sm = es[0]
            for w in range(1, 8):
                sm = sm + es[w]
            inv = 1.0 / sm
            o_t = [None] * 5
            for w in range(8):
                p = es[w] * inv
                vs = vv[16 - 2 * w:48 - 2 * w]
                for tau in range(5):
                    term = p * vs[:, tau * 128:(tau + 1) * 128]
                    o_t[tau] = term if o_t[tau] is None else o_t[tau] + term
            outs.append(jnp.concatenate(o_t, axis=1))
        return jnp.concatenate(outs, axis=0).astype(BF16)

    def b_out_cols(xb, ob, c0, c1):
        return xb[:, c0:c1] + _dot(ob, bwo_ref[:, c0:c1])

    def t3(a):
        return a[:, 0:128], a[:, 128:256], a[:, 256:384]

    def make_att(rows):
        lo = _iota((L, 128), 1) < 64
        r = _iota((rows, 2 * L), 0)
        c = _iota((rows, 2 * L), 1)
        rl = jnp.where(r >= L, 1, 0)
        cl = jnp.where(c >= L, 1, 0)
        rr = r - rl * L
        cc = c - cl * L
        causal = (rr < M) | (rr >= cc)
        left = cl == 0
        diag = rl == cl

        def split_mid(a, swap):
            x0 = jnp.where(lo, a, 0.0)
            x1 = jnp.where(lo, 0.0, a)
            return jnp.concatenate([x1, x0] if swap else [x0, x1], axis=0).astype(BF16)

        def smax(s):
            s = jnp.where(causal, s * scale_a, NEG)
            m_lo = jnp.max(jnp.where(left, s, NEG), axis=1, keepdims=True)
            m_hi = jnp.max(jnp.where(left, NEG, s), axis=1, keepdims=True)
            e = jnp.exp(s - jnp.where(left, m_lo, m_hi))
            s_lo = jnp.sum(jnp.where(left, e, 0.0), axis=1, keepdims=True)
            s_hi = jnp.sum(jnp.where(left, 0.0, e), axis=1, keepdims=True)
            return e * jnp.where(left, 1.0 / s_lo, 1.0 / s_hi)

        if rows == L:
            zero = jnp.zeros((L, 128), F32)

            def scores(q, k):
                q0, qm, q2 = t3(q)
                k0, km, k2 = t3(k)
                r0 = jnp.concatenate([k0, zero], axis=0).astype(BF16)
                r2 = jnp.concatenate([zero, k2], axis=0).astype(BF16)
                return _dot_nt(q0, r0) + _dot_nt(q2, r2) + _dot_nt(qm, split_mid(km, False))

            def pv(p, v):
                v0, vm, v2 = t3(v)
                r0 = jnp.concatenate([v0, zero], axis=0).astype(BF16)
                r2 = jnp.concatenate([zero, v2], axis=0).astype(BF16)
                return jnp.concatenate([_dot(p, r0), _dot(p, split_mid(vm, False)), _dot(p, r2)], axis=1)
        else:
            def scores(q, k):
                q0, qm, q2 = t3(q)
                k0, km, k2 = t3(k)
                k2s = jnp.concatenate([k2[L:2 * L], k2[0:L]], axis=0)
                s0 = _dot_nt(q0, k0.astype(BF16))
                s2 = _dot_nt(q2, k2s.astype(BF16))
                mid = jnp.concatenate([_dot_nt(qm[0:L], split_mid(km[0:L], False)),
                                       _dot_nt(qm[L:2 * L], split_mid(km[L:2 * L], True))], axis=0)
                return jnp.where(diag, s0, s2) + mid

            def pv(p, v):
                v0, vm, v2 = t3(v)
                v2s = jnp.concatenate([v2[L:2 * L], v2[0:L]], axis=0)
                p0 = jnp.where(diag, p, 0.0)
                p1 = jnp.where(diag, 0.0, p)
                o0 = _dot(p0, v0.astype(BF16))
                o2 = _dot(p1, v2s.astype(BF16))
                om = jnp.concatenate([_dot(p[0:L], split_mid(vm[0:L], False)),
                                      _dot(p[L:2 * L], split_mid(vm[L:2 * L], True))], axis=0)
                return jnp.concatenate([o0, om, o2], axis=1)
        return scores, smax, pv

    def a_pass(h, rows, post, first=False, pre_hook=None, mid_hook=None, tail_x=None, tail_y=None):
        scores, smax, pv = make_att(rows)

        def wait(j):
            if first:
                wait_pair(j)
                if j + LOOK < NP:
                    start_pair(j + LOOK)
                if j == NP - 1:
                    cp_xr.start()

        def proj(i, p_ref, j):
            return post(_dot_nt(h, w_ref[j, i]), p_ref, j)

        def outproj(o, j):
            return _dot(o, w_ref[j, 3])

        wait(0)
        q = proj(0, pq_ref, 0)
        k = proj(1, pk_ref, 0)
        v = proj(2, pv_ref, 0)
        if pre_hook is not None:
            pre_hook()
        acc = None
        o_def = None
        for j in range(NP):
            s = scores(q, k)
            if j < NP - 1:
                wait(j + 1)
                qn = proj(0, pq_ref, j + 1)
                kn = proj(1, pk_ref, j + 1)
            else:
                acc = acc + outproj(o_def, j - 1)
                if tail_x is not None:
                    tail_x()
            p = smax(s)
            if j == 8 and mid_hook is not None:
                mid_hook()
            o = pv(p, v)
            if j < NP - 1:
                vn = proj(2, pv_ref, j + 1)
            elif tail_y is not None:
                tail_y()
            if j == NP - 2:
                o_def = o
            else:
                contrib = outproj(o, j)
                acc = contrib if acc is None else acc + contrib
            if j < NP - 1:
                q, k, v = qn, kn, vn
        return acc

    def xseg(s):
        return x_ref[pl.ds(pl.multiple_of(s * SEG, SEG), SEG), :].astype(F32)

    def lxrows(r0, n):
        return lx_ref[pl.ds(pl.multiple_of(r0, 8), n), :]

    def store_out(s, val):
        o_ref[pl.ds(pl.multiple_of(s * SEG, SEG), SEG), :] = val.astype(o_ref.dtype)

    def b_hooks(t, st, extra_mid=None):
        def pre():
            st['xb'], st['bq'] = b_qkv()

        def mid():
            st['ob'] = b_attn(t, st['bq'])
            if extra_mid is not None:
                extra_mid()

        def tx():
            st['xo0'] = b_out_cols(st['xb'], st['ob'], 0, 384)

        def ty():
            st['xo1'] = b_out_cols(st['xb'], st['ob'], 384, 640)
        return dict(pre_hook=pre, mid_hook=mid, tail_x=tx, tail_y=ty)

    def b_finish(st, so):
        xo = jnp.concatenate([st['xo0'], st['xo1']], axis=1)
        x2_scr[...] = xo[0:SEG]
        lx2_scr[...] = _ln(xo[0:SEG])
        store_out(so, xo[SEG:2 * SEG])

    def step_double(t, light):
        st = {}
        xa2 = x2_scr[...]
        mem12 = mem_scr[...]
        lx2 = lx2_scr[...]
        if light:
            rnew = R0 + RN + RN * (t - 2)
            pnew = pl.multiple_of(lax.rem(rnew, PROWS), 8)
            pcur = pl.multiple_of(lax.rem(SEG * (t - 2), PROWS), 8)
            h = jnp.concatenate([mem12, lx2, lxrows(rnew + 2 * SEG, RN)], axis=0)
            if RN % 16 == 0:
                h = h.astype(BF16)
            nxt = (rnew + RN + 2 * SEG, RN)

            def post(a, p_ref, j):
                cols = slice(j * PW, (j + 1) * PW)
                p_ref[pl.ds(pnew, RN), cols] = a[48:48 + RN]
                return jnp.concatenate([a[0:8], p_ref[pl.ds(pcur, SEG), cols], a[8:48]], axis=0)
        else:
            h = jnp.concatenate([mem12.astype(BF16), lxrows(t * SEG, SEG).astype(BF16), lx2.astype(BF16)], axis=0)

            def post(a, p_ref, j):
                return jnp.concatenate([a[0:8], a[16:48], a[8:16], a[48:80]], axis=0)
            nxt = (jnp.minimum(t + 1, nseg - 1) * SEG, SEG)

        def ln_next():
            if nxt[1] % 16 == 0:
                r = pl.ds(pl.multiple_of(nxt[0], 16), nxt[1])
                lx_ref[r, :] = _ln(x_ref[r, :].astype(F32))
            else:
                r0 = (nxt[0] // 16) * 16
                r = pl.ds(pl.multiple_of(r0, 16), 32)
                lx_ref[r, :] = _ln(x_ref[r, :].astype(F32))

        acc = a_pass(h, 2 * L, post, **b_hooks(t, st, ln_next))
        b_finish(st, jnp.maximum(t - 3, 0))
        mem_scr[0:8, :] = acc[0:8]
        mem_scr[8:16, :] = acc[L:L + 8]
        xb_scr[0:SEG, :] = xseg(t) + acc[8:L]
        xb_scr[SEG:2 * SEG, :] = xa2 + acc[L + 8:2 * L]

    def step_single(t, layer, first=False, extra=None):
        st = {}
        if layer == 0:
            xa = x_ref[t * SEG:(t + 1) * SEG, :].astype(F32)
            lxa = lx_ref[t * SEG:(t + 1) * SEG, :]
        else:
            xa = x2_scr[...]
            lxa = lx2_scr[...]
        parts = [mem_scr[layer * 8:layer * 8 + 8, :], lxa]
        if extra is None:
            def post(a, p_ref, j):
                return a
        else:
            e0, en = extra
            parts.append(lx_ref[2 * SEG + e0:2 * SEG + e0 + en, :])

            def post(a, p_ref, j):
                p_ref[e0:e0 + en, j * PW:(j + 1) * PW] = a[L:L + en]
                return a[0:L]
        h = jnp.concatenate(parts, axis=0)
        if first:
            acc = a_pass(h, L, post, first=True)
        else:
            extra_mid = None
            if t == 1:
                def extra_mid():
                    cp_xr.wait()
            acc = a_pass(h, L, post, **b_hooks(t, st, extra_mid))
            b_finish(st, max(t - 3, 0))
        mem_scr[layer * 8:layer * 8 + 8, :] = acc[0:8]
        xb_scr[layer * SEG:(layer + 1) * SEG, :] = xa + acc[8:L]

    perm_all()
    step_single(0, 0, first=True, extra=(0, R0))
    step_single(1, 0, extra=(R0, RN))

    def body_light(t, _):
        step_double(t, True)
        return 0

    def body(t, _):
        step_double(t, False)
        return 0

    lax.fori_loop(2, 2 + NPRE, body_light, 0)
    lax.fori_loop(2 + NPRE, nseg, body, 0)
    step_single(nseg, 1)
    step_single(nseg + 1, 1)
    nh = (nseg - 2) * SEG
    oc0 = pltpu.make_async_copy(o_ref.at[pl.ds(0, nh), :], o_hbm.at[pl.ds(0, nh), :], msem.at[0])
    oc0.start()
    xb, bq = b_qkv()
    ob = b_attn(nseg + 2, bq)
    xo = b_out_cols(xb, ob, 0, D)
    store_out(nseg - 1, xo[SEG:2 * SEG])
    oc1 = pltpu.make_async_copy(o_ref.at[pl.ds(nh, 2 * SEG), :], o_hbm.at[pl.ds(nh, 2 * SEG), :], msem.at[1])
    oc1.start()
    oc0.wait()
    oc1.wait()


@functools.partial(jax.jit, static_argnames=("A_seg_len",))
def pallas_interleave_layers__memory_aug_recurrent_mem_tr__sliding_local_dilated__prompt_kernel(
        A_x, A_mem0, A_Wq, A_Wk, A_Wv, A_Wo, A_seg_len, B_x, B_wqkv, B_wo):
    S = A_x.shape[1]
    x = A_x.reshape(S, D)
    mem0 = A_mem0.reshape(M, D)
    wq = A_Wq.transpose(1, 2, 0).reshape(NP * PW, D)
    wk = A_Wk.transpose(1, 2, 0).reshape(NP * PW, D)
    wv = A_Wv.transpose(1, 2, 0).reshape(NP * PW, D)
    wo = A_Wo.reshape(NP * PW, D)
    anyspec = pl.BlockSpec(memory_space=pl.ANY)
    out = pl.pallas_call(
        functools.partial(_kernel, nseg=S // SEG),
        out_shape=jax.ShapeDtypeStruct((S, D), A_x.dtype),
        in_specs=[anyspec] * 8,
        out_specs=anyspec,
        scratch_shapes=[
            pltpu.VMEM((NP, 4, PW, D), BF16),
            pltpu.VMEM((D, 3 * D), BF16), pltpu.VMEM((D, D), BF16),
            pltpu.VMEM((D, 3 * D), BF16), pltpu.VMEM((D, D), BF16),
            pltpu.VMEM((S, D), BF16), pltpu.VMEM((S, D), BF16), pltpu.VMEM((M, D), BF16),
            pltpu.VMEM((2 * SEG, D), F32),
            pltpu.VMEM((SEG, D), F32), pltpu.VMEM((SEG, D), F32),
            pltpu.VMEM((2 * M, D), F32),
            pltpu.VMEM((2, 16, D), F32), pltpu.VMEM((2, 16, D), F32),
            pltpu.VMEM((PROWS, NP * PW), F32), pltpu.VMEM((PROWS, NP * PW), F32), pltpu.VMEM((PROWS, NP * PW), F32),
            pltpu.VMEM((S, D), F32),
            pltpu.SemaphoreType.DMA((NP,)),
            pltpu.SemaphoreType.DMA((5,)),
        ],
        compiler_params=pltpu.CompilerParams(vmem_limit_bytes=100 * 1024 * 1024),
    )(x, mem0, wq, wk, wv, wo, B_wqkv, B_wo)
    return out.reshape(A_x.shape)
```

```python
import functools
import numpy as np
import jax
import jax.numpy as jnp
from jax import lax
import jax.experimental.pallas as pl
import jax.experimental.pallas.tpu as pltpu

F32 = jnp.float32
BF16 = jnp.bfloat16

SEG, M, D = 32, 8, 640
L = M + SEG
NP = 16
PW = 384
NEG = -1e9
RN = 16
PROWS = 416
R0 = 368
NPRE = (R0 + RN - SEG) // (SEG - RN) + 1
LOOK = 3
WGRP = "1111111111111111"
LOOK0 = 1
BPOS = 4
PERM0 = 8
PSTEP = 2
assert R0 % RN == 0 and R0 + 2 * RN <= PROWS and PROWS % RN == 0 and PROWS % SEG == 0


def _ln(x):
    m = jnp.mean(x, axis=-1, keepdims=True)
    xc = x - m
    v = jnp.mean(xc * xc, axis=-1, keepdims=True)
    return xc * lax.rsqrt(v + 1e-5)


def _dot(a, b):
    return jnp.dot(a, b, preferred_element_type=F32)


def _dot_nt(a, b):
    return lax.dot_general(a, b, (((1,), (1,)), ((), ())), preferred_element_type=F32)


def _iota(shape, dim):
    return lax.broadcasted_iota(jnp.int32, shape, dim)


def _kernel(x_hbm, mem0_hbm, wq_hbm, wk_hbm, wv_hbm, wo_hbm, bqkv_hbm, bwo_hbm, o_hbm,
            w_ref, braw_ref, bworaw_ref, bqkv_ref, bwo_ref, x_ref, o_ref, mem0_ref,
            xb_scr, x2_scr, lx2_scr, mem_scr, kprev_scr, vprev_scr,
            pq_ref, pk_ref, pv_ref, lx_ref, wn_ref, ptmp, wsem, msem, *, nseg):
    S_ROWS = nseg * SEG
    XH = 2 * SEG + R0 + SEG
    scale_a = 192 ** -0.5
    scale_b = 20 ** -0.5

    def wcopies(j):
        sl = pl.ds(j * PW, PW)
        return [pltpu.make_async_copy(hbm.at[sl, :], w_ref.at[j, i], wsem.at[j])
                for i, hbm in enumerate((wq_hbm, wk_hbm, wv_hbm, wo_hbm))]

    def start_pair(j):
        for c in wcopies(j):
            c.start()

    def wait_pair(j):
        pltpu.make_async_copy(w_ref.at[j], w_ref.at[j], wsem.at[j]).wait()

    cp_b = [pltpu.make_async_copy(bqkv_hbm.at[:, pl.ds(i * D, D)], braw_ref.at[i], msem.at[5 + i]) for i in range(3)]
    cp_bwo = pltpu.make_async_copy(bwo_hbm, bworaw_ref, msem.at[1])
    cp_xh = pltpu.make_async_copy(x_hbm.at[pl.ds(0, XH), :], x_ref.at[pl.ds(0, XH), :], msem.at[2])
    cp_mem = pltpu.make_async_copy(mem0_hbm, mem0_ref, msem.at[3])
    cp_xr = pltpu.make_async_copy(x_hbm.at[pl.ds(XH, S_ROWS - XH), :], x_ref.at[pl.ds(XH, S_ROWS - XH), :], msem.at[4])

    cp_xh.start()
    cp_mem.start()
    for j in range(LOOK0):
        start_pair(j)

    xb_scr[...] = jnp.zeros_like(xb_scr)
    x2_scr[...] = jnp.zeros_like(x2_scr)
    lx2_scr[...] = jnp.zeros_like(lx2_scr)
    kprev_scr[...] = jnp.zeros_like(kprev_scr)
    vprev_scr[...] = jnp.zeros_like(vprev_scr)
    cp_xh.wait()
    cp_mem.wait()
    lx_ref[0:XH, :] = _ln(x_ref[0:XH, :].astype(F32))
    mem0 = mem0_ref[...].astype(F32)
    mem_scr[0:8, :] = mem0
    mem_scr[8:16, :] = mem0

    def perm_qkv_a(part):
        for kt in range(5):
            ptmp[kt] = braw_ref[part, kt * 128:(kt + 1) * 128, :].astype(F32).T

    def perm_qkv_b(part):
        for nt in range(5):
            for kt in range(5):
                rows = jnp.concatenate([ptmp[kt, pl.ds(4 * nt + g, 32, stride=20), :] for g in range(4)], axis=0)
                bqkv_ref[kt * 128:(kt + 1) * 128, part * D + nt * 128:part * D + (nt + 1) * 128] = rows.T.astype(BF16)

    def perm_wo():
        for ct in range(5):
            ptmp[ct] = bworaw_ref[:, ct * 128:(ct + 1) * 128].astype(F32)
        for d in range(20):
            for ct in range(5):
                bwo_ref[d * 32:(d + 1) * 32, ct * 128:(ct + 1) * 128] = ptmp[ct, pl.ds(d, 32, stride=20), :].astype(BF16)

    perm_pieces = [functools.partial(f, part) for part in range(3) for f in (perm_qkv_a, perm_qkv_b)] + [perm_wo]

    def b_qkv():
        xb = xb_scr[...]
        hb = _ln(xb).astype(BF16)
        return xb, _dot(hb, bqkv_ref[...])

    def b_attn(t, qkv):
        row = _iota((SEG, 128), 0)
        outs = []
        for l in range(2):
            seg = t - 1 - 2 * l
            q = qkv[l * SEG:(l + 1) * SEG, 0:D]
            k = qkv[l * SEG:(l + 1) * SEG, D:2 * D]
            v = qkv[l * SEG:(l + 1) * SEG, 2 * D:3 * D]
            kk = jnp.concatenate([kprev_scr[l], k], axis=0)
            vv = jnp.concatenate([vprev_scr[l], v], axis=0)
            kprev_scr[l] = k[16:32]
            vprev_scr[l] = v[16:32]
            logits = []
            for w in range(8):
                ks = kk[16 - 2 * w:48 - 2 * w]
                y = q[:, 0:128] * ks[:, 0:128]
                for tau in range(1, 5):
                    y = y + q[:, tau * 128:(tau + 1) * 128] * ks[:, tau * 128:(tau + 1) * 128]
                y = y + pltpu.roll(y, 64, 1)
                y = y + pltpu.roll(y, 32, 1)
                valid = (seg * SEG + row - 2 * w) >= 0
                logits.append(jnp.where(valid, y * scale_b, NEG))
            mx = logits[0]
            for w in range(1, 8):
                mx = jnp.maximum(mx, logits[w])
            es = [jnp.exp(lg - mx) for lg in logits]
            sm = es[0]
            for w in range(1, 8):
                sm = sm + es[w]
            inv = 1.0 / sm
            o_t = [None] * 5
            for w in range(8):
                p = es[w] * inv
                vs = vv[16 - 2 * w:48 - 2 * w]
                for tau in range(5):
                    term = p * vs[:, tau * 128:(tau + 1) * 128]
                    o_t[tau] = term if o_t[tau] is None else o_t[tau] + term
            outs.append(jnp.concatenate(o_t, axis=1))
        return jnp.concatenate(outs, axis=0).astype(BF16)

    def b_out_cols(xb, ob, c0, c1):
        return xb[:, c0:c1] + _dot(ob, bwo_ref[:, c0:c1])

    def t3(a):
        return a[:, 0:128], a[:, 128:256], a[:, 256:384]

    def make_att(rows):
        lo = _iota((L, 128), 1) < 64
        r = _iota((rows, 2 * L), 0)
        c = _iota((rows, 2 * L), 1)
        rl = jnp.where(r >= L, 1, 0)
        cl = jnp.where(c >= L, 1, 0)
        rr = r - rl * L
        cc = c - cl * L
        causal = (rr < M) | (rr >= cc)
        left = cl == 0
        diag = rl == cl

        def split_mid(a, swap):
            x0 = jnp.where(lo, a, 0.0)
            x1 = jnp.where(lo, 0.0, a)
            return jnp.concatenate([x1, x0] if swap else [x0, x1], axis=0).astype(BF16)

        def smax(s):
            s = jnp.where(causal, s * scale_a, NEG)
            m_lo = jnp.max(jnp.where(left, s, NEG), axis=1, keepdims=True)
            m_hi = jnp.max(jnp.where(left, NEG, s), axis=1, keepdims=True)
            e = jnp.exp(s - jnp.where(left, m_lo, m_hi))
            s_lo = jnp.sum(jnp.where(left, e, 0.0), axis=1, keepdims=True)
            s_hi = jnp.sum(jnp.where(left, 0.0, e), axis=1, keepdims=True)
            return e * jnp.where(left, 1.0 / s_lo, 1.0 / s_hi)

        if rows == L:
            zero = jnp.zeros((L, 128), F32)

            def scores(q, k):
                q0, qm, q2 = t3(q)
                k0, km, k2 = t3(k)
                r0 = jnp.concatenate([k0, zero], axis=0).astype(BF16)
                r2 = jnp.concatenate([zero, k2], axis=0).astype(BF16)
                return _dot_nt(q0, r0) + _dot_nt(q2, r2) + _dot_nt(qm, split_mid(km, False))

            def pv(p, v):
                v0, vm, v2 = t3(v)
                r0 = jnp.concatenate([v0, zero], axis=0).astype(BF16)
                r2 = jnp.concatenate([zero, v2], axis=0).astype(BF16)
                return jnp.concatenate([_dot(p, r0), _dot(p, split_mid(vm, False)), _dot(p, r2)], axis=1)
        else:
            def scores(q, k):
                q0, qm, q2 = t3(q)
                k0, km, k2 = t3(k)
                k2s = jnp.concatenate([k2[L:2 * L], k2[0:L]], axis=0)
                s0 = _dot_nt(q0, k0.astype(BF16))
                s2 = _dot_nt(q2, k2s.astype(BF16))
                mid = jnp.concatenate([_dot_nt(qm[0:L], split_mid(km[0:L], False)),
                                       _dot_nt(qm[L:2 * L], split_mid(km[L:2 * L], True))], axis=0)
                return jnp.where(diag, s0, s2) + mid

            def pv(p, v):
                v0, vm, v2 = t3(v)
                v2s = jnp.concatenate([v2[L:2 * L], v2[0:L]], axis=0)
                p0 = jnp.where(diag, p, 0.0)
                p1 = jnp.where(diag, 0.0, p)
                o0 = _dot(p0, v0.astype(BF16))
                o2 = _dot(p1, v2s.astype(BF16))
                om = jnp.concatenate([_dot(p[0:L], split_mid(vm[0:L], False)),
                                      _dot(p[L:2 * L], split_mid(vm[L:2 * L], True))], axis=0)
                return jnp.concatenate([o0, om, o2], axis=1)
        return scores, smax, pv

    def a_pass(h, rows, post, first=False, pre_hook=None, mid_hook=None, tail_x=None, tail_y=None):
        scores, smax, pv = make_att(rows)
        started = [LOOK0]

        def wait(j):
            if first:
                if WGRP[j] == "1":
                    jj = j
                    wait_pair(jj)
                    while jj + 1 < NP and WGRP[jj + 1] == "0":
                        jj += 1
                        wait_pair(jj)
                    for js in range(started[0], min(NP, jj + 1 + LOOK)):
                        start_pair(js)
                        started[0] = js + 1
                    if j <= BPOS <= jj:
                        for c in cp_b + [cp_bwo]:
                            c.start()
                    if j <= PERM0 + 1 <= jj:
                        for c in cp_b + [cp_bwo]:
                            c.wait()
                    if jj == NP - 1:
                        cp_xr.start()

        def proj(i, p_ref, j):
            if first:
                return post(_dot_nt(h, w_ref[j, i]), p_ref, j)
            return post(_dot(h, wn_ref[j, i]), p_ref, j)

        def outproj(o, j):
            return _dot(o, w_ref[j, 3])

        wait(0)
        q = proj(0, pq_ref, 0)
        k = proj(1, pk_ref, 0)
        v = proj(2, pv_ref, 0)
        if pre_hook is not None:
            pre_hook()
        acc = None
        o_def = None
        for j in range(NP):
            s = scores(q, k)
            if j < NP - 1:
                wait(j + 1)
                qn = proj(0, pq_ref, j + 1)
                kn = proj(1, pk_ref, j + 1)
            else:
                acc = acc + outproj(o_def, j - 1)
                if tail_x is not None:
                    tail_x()
            p = smax(s)
            if j == 8 and mid_hook is not None:
                mid_hook()
            o = pv(p, v)
            if j < NP - 1:
                vn = proj(2, pv_ref, j + 1)
            elif tail_y is not None:
                tail_y()
            if j == NP - 2:
                o_def = o
            else:
                contrib = outproj(o, j)
                acc = contrib if acc is None else acc + contrib
            if first and PERM0 <= j < PERM0 + len(perm_pieces):
                perm_pieces[j - PERM0]()
            if first:
                for i in range(3):
                    wn_ref[j, i] = w_ref[j, i].T
            if j < NP - 1:
                q, k, v = qn, kn, vn
        return acc

    def xseg(s):
        return x_ref[pl.ds(pl.multiple_of(s * SEG, SEG), SEG), :].astype(F32)

    def lxrows(r0, n):
        return lx_ref[pl.ds(pl.multiple_of(r0, 8), n), :]

    def store_out(s, val):
        o_ref[pl.ds(pl.multiple_of(s * SEG, SEG), SEG), :] = val.astype(o_ref.dtype)

    def b_hooks(t, st, extra_mid=None):
        def pre():
            st['xb'], st['bq'] = b_qkv()

        def mid():
            st['ob'] = b_attn(t, st['bq'])
            if extra_mid is not None:
                extra_mid()

        def tx():
            st['xo0'] = b_out_cols(st['xb'], st['ob'], 0, 384)

        def ty():
            st['xo1'] = b_out_cols(st['xb'], st['ob'], 384, 640)
        return dict(pre_hook=pre, mid_hook=mid, tail_x=tx, tail_y=ty)

    def b_finish(st, so):
        xo = jnp.concatenate([st['xo0'], st['xo1']], axis=1)
        x2_scr[...] = xo[0:SEG]
        lx2_scr[...] = _ln(xo[0:SEG])
        store_out(so, xo[SEG:2 * SEG])

    def step_double(t, light):
        st = {}
        xa2 = x2_scr[...]
        mem12 = mem_scr[...]
        lx2 = lx2_scr[...]
        if light:
            rnew = R0 + RN + RN * (t - 2)
            pnew = pl.multiple_of(lax.rem(rnew, PROWS), 8)
            pcur = pl.multiple_of(lax.rem(SEG * (t - 2), PROWS), 8)
            h = jnp.concatenate([mem12, lx2, lxrows(rnew + 2 * SEG, RN)], axis=0)
            if RN % 16 == 0:
                h = h.astype(BF16)
            nxt = (rnew + RN + 2 * SEG, RN)

            def post(a, p_ref, j):
                cols = slice(j * PW, (j + 1) * PW)
                p_ref[pl.ds(pnew, RN), cols] = a[48:48 + RN]
                return jnp.concatenate([a[0:8], p_ref[pl.ds(pcur, SEG), cols], a[8:48]], axis=0)
        else:
            h = jnp.concatenate([mem12.astype(BF16), lxrows(t * SEG, SEG).astype(BF16), lx2.astype(BF16)], axis=0)

            def post(a, p_ref, j):
                return jnp.concatenate([a[0:8], a[16:48], a[8:16], a[48:80]], axis=0)
            nxt = (jnp.minimum(t + 1, nseg - 1) * SEG, SEG)

        def ln_next():
            if nxt[1] % 16 == 0:
                r = pl.ds(pl.multiple_of(nxt[0], 16), nxt[1])
                lx_ref[r, :] = _ln(x_ref[r, :].astype(F32))
            else:
                r0 = (nxt[0] // 16) * 16
                r = pl.ds(pl.multiple_of(r0, 16), 32)
                lx_ref[r, :] = _ln(x_ref[r, :].astype(F32))

        acc = a_pass(h, 2 * L, post, **b_hooks(t, st, ln_next))
        b_finish(st, jnp.maximum(t - 3, 0))
        mem_scr[0:8, :] = acc[0:8]
        mem_scr[8:16, :] = acc[L:L + 8]
        xb_scr[0:SEG, :] = xseg(t) + acc[8:L]
        xb_scr[SEG:2 * SEG, :] = xa2 + acc[L + 8:2 * L]

    def step_single(t, layer, first=False, extra=None):
        st = {}
        if layer == 0:
            xa = x_ref[t * SEG:(t + 1) * SEG, :].astype(F32)
            lxa = lx_ref[t * SEG:(t + 1) * SEG, :]
        else:
            xa = x2_scr[...]
            lxa = lx2_scr[...]
        parts = [mem_scr[layer * 8:layer * 8 + 8, :], lxa]
        if extra is None:
            def post(a, p_ref, j):
                return a
        else:
            e0, en = extra
            parts.append(lx_ref[2 * SEG + e0:2 * SEG + e0 + en, :])

            def post(a, p_ref, j):
                p_ref[e0:e0 + en, j * PW:(j + 1) * PW] = a[L:L + en]
                return a[0:L]
        h = jnp.concatenate(parts, axis=0)
        if first:
            acc = a_pass(h, L, post, first=True)
        else:
            extra_mid = None
            if t == 1:
                def extra_mid():
                    cp_xr.wait()
            acc = a_pass(h, L, post, **b_hooks(t, st, extra_mid))
            b_finish(st, max(t - 3, 0))
        mem_scr[layer * 8:layer * 8 + 8, :] = acc[0:8]
        xb_scr[layer * SEG:(layer + 1) * SEG, :] = xa + acc[8:L]

    step_single(0, 0, first=True, extra=(0, R0))
    step_single(1, 0, extra=(R0, RN))

    def body_light(t, _):
        step_double(t, True)
        return 0

    def body(t, _):
        step_double(t, False)
        return 0

    lax.fori_loop(2, 2 + NPRE, body_light, 0)
    lax.fori_loop(2 + NPRE, nseg, body, 0)
    step_single(nseg, 1)
    step_single(nseg + 1, 1)
    nh = (nseg - 2) * SEG
    oc0 = pltpu.make_async_copy(o_ref.at[pl.ds(0, nh), :], o_hbm.at[pl.ds(0, nh), :], msem.at[0])
    oc0.start()
    xb, bq = b_qkv()
    ob = b_attn(nseg + 2, bq)
    xo = b_out_cols(xb, ob, 0, D)
    store_out(nseg - 1, xo[SEG:2 * SEG])
    oc1 = pltpu.make_async_copy(o_ref.at[pl.ds(nh, 2 * SEG), :], o_hbm.at[pl.ds(nh, 2 * SEG), :], msem.at[5])
    oc1.start()
    oc0.wait()
    oc1.wait()


@functools.partial(jax.jit, static_argnames=("A_seg_len",))
def pallas_interleave_layers__memory_aug_recurrent_mem_tr__sliding_local_dilated__prompt_kernel(
        A_x, A_mem0, A_Wq, A_Wk, A_Wv, A_Wo, A_seg_len, B_x, B_wqkv, B_wo):
    S = A_x.shape[1]
    x = A_x.reshape(S, D)
    mem0 = A_mem0.reshape(M, D)
    wq = A_Wq.transpose(1, 2, 0).reshape(NP * PW, D)
    wk = A_Wk.transpose(1, 2, 0).reshape(NP * PW, D)
    wv = A_Wv.transpose(1, 2, 0).reshape(NP * PW, D)
    wo = A_Wo.reshape(NP * PW, D)
    anyspec = pl.BlockSpec(memory_space=pl.ANY)
    out = pl.pallas_call(
        functools.partial(_kernel, nseg=S // SEG),
        out_shape=jax.ShapeDtypeStruct((S, D), A_x.dtype),
        in_specs=[anyspec] * 8,
        out_specs=anyspec,
        scratch_shapes=[
            pltpu.VMEM((NP, 4, PW, D), BF16),
            pltpu.VMEM((3, D, D), BF16), pltpu.VMEM((D, D), BF16),
            pltpu.VMEM((D, 3 * D), BF16), pltpu.VMEM((D, D), BF16),
            pltpu.VMEM((S, D), BF16), pltpu.VMEM((S, D), BF16), pltpu.VMEM((M, D), BF16),
            pltpu.VMEM((2 * SEG, D), F32),
            pltpu.VMEM((SEG, D), F32), pltpu.VMEM((SEG, D), F32),
            pltpu.VMEM((2 * M, D), F32),
            pltpu.VMEM((2, 16, D), F32), pltpu.VMEM((2, 16, D), F32),
            pltpu.VMEM((PROWS, NP * PW), F32), pltpu.VMEM((PROWS, NP * PW), F32), pltpu.VMEM((PROWS, NP * PW), F32),
            pltpu.VMEM((S, D), F32),
            pltpu.VMEM((NP, 3, D, PW), BF16),
            pltpu.VMEM((5, D, 128), F32),
            pltpu.SemaphoreType.DMA((NP,)),
            pltpu.SemaphoreType.DMA((8,)),
        ],
        compiler_params=pltpu.CompilerParams(vmem_limit_bytes=118 * 1024 * 1024),
    )(x, mem0, wq, wk, wv, wo, B_wqkv, B_wo)
    return out.reshape(A_x.shape)
```

```python
import functools
import numpy as np
import jax
import jax.numpy as jnp
from jax import lax
import jax.experimental.pallas as pl
import jax.experimental.pallas.tpu as pltpu

F32 = jnp.float32
BF16 = jnp.bfloat16

SEG, M, D = 32, 8, 640
L = M + SEG
NP = 16
PW = 384
NEG = -1e9
RN = 16
PROWS = 416
R0 = 368
NPRE = (R0 + RN - SEG) // (SEG - RN) + 1
LOOK = 3
WGRP = "1111111111111111"
LOOK0 = 1
BPOS = 4
PERM0 = 8
PSTEP = 2
assert R0 % RN == 0 and R0 + 2 * RN <= PROWS and PROWS % RN == 0 and PROWS % SEG == 0


def _ln(x):
    m = jnp.mean(x, axis=-1, keepdims=True)
    xc = x - m
    v = jnp.mean(xc * xc, axis=-1, keepdims=True)
    return xc * lax.rsqrt(v + 1e-5)


def _dot(a, b):
    return jnp.dot(a, b, preferred_element_type=F32)


def _dot_nt(a, b):
    return lax.dot_general(a, b, (((1,), (1,)), ((), ())), preferred_element_type=F32)


def _iota(shape, dim):
    return lax.broadcasted_iota(jnp.int32, shape, dim)


def _kernel(x_hbm, mem0_hbm, wq_hbm, wk_hbm, wv_hbm, wo_hbm, bqkv_hbm, bwo_hbm, o_hbm,
            w_ref, braw_ref, bworaw_ref, bqkv_ref, bwo_ref, x_ref, o_ref, mem0_ref,
            xb_scr, x2_scr, lx2_scr, mem_scr, kprev_scr, vprev_scr,
            pq_ref, pk_ref, pv_ref, lx_ref, wn_ref, ptmp, wsem, msem, *, nseg):
    S_ROWS = nseg * SEG
    XH = 2 * SEG + R0 + SEG
    scale_a = 192 ** -0.5
    scale_b = 20 ** -0.5

    def wcopies(j):
        sl = pl.ds(j * PW, PW)
        return [pltpu.make_async_copy(hbm.at[sl, :], w_ref.at[j, i], wsem.at[j])
                for i, hbm in enumerate((wq_hbm, wk_hbm, wv_hbm, wo_hbm))]

    def start_pair(j):
        for c in wcopies(j):
            c.start()

    def wait_pair(j):
        pltpu.make_async_copy(w_ref.at[j], w_ref.at[j], wsem.at[j]).wait()

    cp_b = [pltpu.make_async_copy(bqkv_hbm.at[:, pl.ds(i * D, D)], braw_ref.at[i], msem.at[5 + i]) for i in range(3)]
    cp_bwo = pltpu.make_async_copy(bwo_hbm, bworaw_ref, msem.at[1])
    cp_xh = pltpu.make_async_copy(x_hbm.at[pl.ds(0, XH), :], x_ref.at[pl.ds(0, XH), :], msem.at[2])
    cp_mem = pltpu.make_async_copy(mem0_hbm, mem0_ref, msem.at[3])
    cp_xr = pltpu.make_async_copy(x_hbm.at[pl.ds(XH, S_ROWS - XH), :], x_ref.at[pl.ds(XH, S_ROWS - XH), :], msem.at[4])

    cp_xh.start()
    cp_mem.start()
    for j in range(LOOK0):
        start_pair(j)

    xb_scr[...] = jnp.zeros_like(xb_scr)
    x2_scr[...] = jnp.zeros_like(x2_scr)
    lx2_scr[...] = jnp.zeros_like(lx2_scr)
    kprev_scr[...] = jnp.zeros_like(kprev_scr)
    vprev_scr[...] = jnp.zeros_like(vprev_scr)
    cp_xh.wait()
    cp_mem.wait()
    lx_ref[0:XH, :] = _ln(x_ref[0:XH, :].astype(F32))
    mem0 = mem0_ref[...].astype(F32)
    mem_scr[0:8, :] = mem0
    mem_scr[8:16, :] = mem0

    def perm_qkv_a(part):
        for kt in range(5):
            ptmp[kt] = braw_ref[part, kt * 128:(kt + 1) * 128, :].astype(F32).T

    def perm_qkv_b(part):
        for nt in range(5):
            for kt in range(5):
                rows = jnp.concatenate([ptmp[kt, pl.ds(4 * nt + g, 32, stride=20), :] for g in range(4)], axis=0)
                bqkv_ref[kt * 128:(kt + 1) * 128, part * D + nt * 128:part * D + (nt + 1) * 128] = rows.T.astype(BF16)

    def perm_wo():
        for ct in range(5):
            ptmp[ct] = bworaw_ref[:, ct * 128:(ct + 1) * 128].astype(F32)
        for d in range(20):
            for ct in range(5):
                bwo_ref[d * 32:(d + 1) * 32, ct * 128:(ct + 1) * 128] = ptmp[ct, pl.ds(d, 32, stride=20), :].astype(BF16)

    perm_pieces = [functools.partial(f, part) for part in range(3) for f in (perm_qkv_a, perm_qkv_b)] + [perm_wo]

    def b_qkv(ls):
        xb = xb_scr[ls[0] * SEG:(ls[-1] + 1) * SEG, :]
        hb = _ln(xb).astype(BF16)
        return xb, _dot(hb, bqkv_ref[...])

    def b_attn(t, qkv, ls):
        row = _iota((SEG, 128), 0)
        outs = []
        for i, l in enumerate(ls):
            seg = t - 1 - 2 * l
            q = qkv[i * SEG:(i + 1) * SEG, 0:D]
            k = qkv[i * SEG:(i + 1) * SEG, D:2 * D]
            v = qkv[i * SEG:(i + 1) * SEG, 2 * D:3 * D]
            kk = jnp.concatenate([kprev_scr[l], k], axis=0)
            vv = jnp.concatenate([vprev_scr[l], v], axis=0)
            kprev_scr[l] = k[16:32]
            vprev_scr[l] = v[16:32]
            logits = []
            for w in range(8):
                ks = kk[16 - 2 * w:48 - 2 * w]
                y = q[:, 0:128] * ks[:, 0:128]
                for tau in range(1, 5):
                    y = y + q[:, tau * 128:(tau + 1) * 128] * ks[:, tau * 128:(tau + 1) * 128]
                y = y + pltpu.roll(y, 64, 1)
                y = y + pltpu.roll(y, 32, 1)
                valid = (seg * SEG + row - 2 * w) >= 0
                logits.append(jnp.where(valid, y * scale_b, NEG))
            mx = logits[0]
            for w in range(1, 8):
                mx = jnp.maximum(mx, logits[w])
            es = [jnp.exp(lg - mx) for lg in logits]
            sm = es[0]
            for w in range(1, 8):
                sm = sm + es[w]
            inv = 1.0 / sm
            o_t = [None] * 5
            for w in range(8):
                p = es[w] * inv
                vs = vv[16 - 2 * w:48 - 2 * w]
                for tau in range(5):
                    term = p * vs[:, tau * 128:(tau + 1) * 128]
                    o_t[tau] = term if o_t[tau] is None else o_t[tau] + term
            outs.append(jnp.concatenate(o_t, axis=1))
        return jnp.concatenate(outs, axis=0).astype(BF16)

    def b_out_cols(xb, ob, c0, c1):
        return xb[:, c0:c1] + _dot(ob, bwo_ref[:, c0:c1])

    def t3(a):
        return a[:, 0:128], a[:, 128:256], a[:, 256:384]

    def make_att(rows):
        lo = _iota((L, 128), 1) < 64
        r = _iota((rows, 2 * L), 0)
        c = _iota((rows, 2 * L), 1)
        rl = jnp.where(r >= L, 1, 0)
        cl = jnp.where(c >= L, 1, 0)
        rr = r - rl * L
        cc = c - cl * L
        causal = (rr < M) | (rr >= cc)
        left = cl == 0
        diag = rl == cl

        def split_mid(a, swap):
            x0 = jnp.where(lo, a, 0.0)
            x1 = jnp.where(lo, 0.0, a)
            return jnp.concatenate([x1, x0] if swap else [x0, x1], axis=0).astype(BF16)

        def smax(s):
            s = jnp.where(causal, s * scale_a, NEG)
            m_lo = jnp.max(jnp.where(left, s, NEG), axis=1, keepdims=True)
            m_hi = jnp.max(jnp.where(left, NEG, s), axis=1, keepdims=True)
            e = jnp.exp(s - jnp.where(left, m_lo, m_hi))
            s_lo = jnp.sum(jnp.where(left, e, 0.0), axis=1, keepdims=True)
            s_hi = jnp.sum(jnp.where(left, 0.0, e), axis=1, keepdims=True)
            return e * jnp.where(left, 1.0 / s_lo, 1.0 / s_hi)

        if rows == L:
            zero = jnp.zeros((L, 128), F32)

            def scores(q, k):
                q0, qm, q2 = t3(q)
                k0, km, k2 = t3(k)
                r0 = jnp.concatenate([k0, zero], axis=0).astype(BF16)
                r2 = jnp.concatenate([zero, k2], axis=0).astype(BF16)
                return _dot_nt(q0, r0) + _dot_nt(q2, r2) + _dot_nt(qm, split_mid(km, False))

            def pv(p, v):
                v0, vm, v2 = t3(v)
                r0 = jnp.concatenate([v0, zero], axis=0).astype(BF16)
                r2 = jnp.concatenate([zero, v2], axis=0).astype(BF16)
                return jnp.concatenate([_dot(p, r0), _dot(p, split_mid(vm, False)), _dot(p, r2)], axis=1)
        else:
            def scores(q, k):
                q0, qm, q2 = t3(q)
                k0, km, k2 = t3(k)
                k2s = jnp.concatenate([k2[L:2 * L], k2[0:L]], axis=0)
                s0 = _dot_nt(q0, k0.astype(BF16))
                s2 = _dot_nt(q2, k2s.astype(BF16))
                mid = jnp.concatenate([_dot_nt(qm[0:L], split_mid(km[0:L], False)),
                                       _dot_nt(qm[L:2 * L], split_mid(km[L:2 * L], True))], axis=0)
                return jnp.where(diag, s0, s2) + mid

            def pv(p, v):
                v0, vm, v2 = t3(v)
                v2s = jnp.concatenate([v2[L:2 * L], v2[0:L]], axis=0)
                p0 = jnp.where(diag, p, 0.0)
                p1 = jnp.where(diag, 0.0, p)
                o0 = _dot(p0, v0.astype(BF16))
                o2 = _dot(p1, v2s.astype(BF16))
                om = jnp.concatenate([_dot(p[0:L], split_mid(vm[0:L], False)),
                                      _dot(p[L:2 * L], split_mid(vm[L:2 * L], True))], axis=0)
                return jnp.concatenate([o0, om, o2], axis=1)
        return scores, smax, pv

    def a_pass(h, rows, post, first=False, pre_hook=None, mid_hook=None, tail_x=None, tail_y=None):
        scores, smax, pv = make_att(rows)
        started = [LOOK0]

        def wait(j):
            if first:
                if WGRP[j] == "1":
                    jj = j
                    wait_pair(jj)
                    while jj + 1 < NP and WGRP[jj + 1] == "0":
                        jj += 1
                        wait_pair(jj)
                    for js in range(started[0], min(NP, jj + 1 + LOOK)):
                        start_pair(js)
                        started[0] = js + 1
                    if j <= BPOS <= jj:
                        for c in cp_b + [cp_bwo]:
                            c.start()
                    if j <= PERM0 + 1 <= jj:
                        for c in cp_b + [cp_bwo]:
                            c.wait()
                    if jj == NP - 1:
                        cp_xr.start()

        def proj(i, p_ref, j):
            if first:
                return post(_dot_nt(h, w_ref[j, i]), p_ref, j)
            return post(_dot(h, wn_ref[j, i]), p_ref, j)

        def outproj(o, j):
            return _dot(o, w_ref[j, 3])

        wait(0)
        q = proj(0, pq_ref, 0)
        k = proj(1, pk_ref, 0)
        v = proj(2, pv_ref, 0)
        if pre_hook is not None:
            pre_hook()
        acc = None
        o_def = None
        for j in range(NP):
            s = scores(q, k)
            if j < NP - 1:
                wait(j + 1)
                qn = proj(0, pq_ref, j + 1)
                kn = proj(1, pk_ref, j + 1)
            else:
                acc = acc + outproj(o_def, j - 1)
                if tail_x is not None:
                    tail_x()
            p = smax(s)
            if j == 8 and mid_hook is not None:
                mid_hook()
            o = pv(p, v)
            if j < NP - 1:
                vn = proj(2, pv_ref, j + 1)
            elif tail_y is not None:
                tail_y()
            if j == NP - 2:
                o_def = o
            else:
                contrib = outproj(o, j)
                acc = contrib if acc is None else acc + contrib
            if first and PERM0 <= j < PERM0 + len(perm_pieces):
                perm_pieces[j - PERM0]()
            if first:
                for i in range(3):
                    wn_ref[j, i] = w_ref[j, i].T
            if j < NP - 1:
                q, k, v = qn, kn, vn
        return acc

    def xseg(s):
        return x_ref[pl.ds(pl.multiple_of(s * SEG, SEG), SEG), :].astype(F32)

    def lxrows(r0, n):
        return lx_ref[pl.ds(pl.multiple_of(r0, 8), n), :]

    def store_out(s, val):
        o_ref[pl.ds(pl.multiple_of(s * SEG, SEG), SEG), :] = val.astype(o_ref.dtype)

    def b_hooks(t, st, extra_mid=None, ls=(0, 1)):
        def pre():
            st['xb'], st['bq'] = b_qkv(ls)

        def mid():
            st['ob'] = b_attn(t, st['bq'], ls)
            if extra_mid is not None:
                extra_mid()

        def tx():
            st['xo0'] = b_out_cols(st['xb'], st['ob'], 0, 384)

        def ty():
            st['xo1'] = b_out_cols(st['xb'], st['ob'], 384, 640)
        return dict(pre_hook=pre, mid_hook=mid, tail_x=tx, tail_y=ty)

    def b_finish(st, so, ls=(0, 1)):
        xo = jnp.concatenate([st['xo0'], st['xo1']], axis=1)
        if 0 in ls:
            x2_scr[...] = xo[0:SEG]
            lx2_scr[...] = _ln(xo[0:SEG])
        if 1 in ls:
            store_out(so, xo[(len(ls) - 1) * SEG:len(ls) * SEG])

    def step_double(t, light):
        st = {}
        xa2 = x2_scr[...]
        mem12 = mem_scr[...]
        lx2 = lx2_scr[...]
        if light:
            rnew = R0 + RN + RN * (t - 2)
            pnew = pl.multiple_of(lax.rem(rnew, PROWS), 8)
            pcur = pl.multiple_of(lax.rem(SEG * (t - 2), PROWS), 8)
            h = jnp.concatenate([mem12, lx2, lxrows(rnew + 2 * SEG, RN)], axis=0)
            if RN % 16 == 0:
                h = h.astype(BF16)
            nxt = (rnew + RN + 2 * SEG, RN)

            def post(a, p_ref, j):
                cols = slice(j * PW, (j + 1) * PW)
                p_ref[pl.ds(pnew, RN), cols] = a[48:48 + RN]
                return jnp.concatenate([a[0:8], p_ref[pl.ds(pcur, SEG), cols], a[8:48]], axis=0)
        else:
            h = jnp.concatenate([mem12.astype(BF16), lxrows(t * SEG, SEG).astype(BF16), lx2.astype(BF16)], axis=0)

            def post(a, p_ref, j):
                return jnp.concatenate([a[0:8], a[16:48], a[8:16], a[48:80]], axis=0)
            nxt = (jnp.minimum(t + 1, nseg - 1) * SEG, SEG)

        def ln_next():
            if nxt[1] % 16 == 0:
                r = pl.ds(pl.multiple_of(nxt[0], 16), nxt[1])
                lx_ref[r, :] = _ln(x_ref[r, :].astype(F32))
            else:
                r0 = (nxt[0] // 16) * 16
                r = pl.ds(pl.multiple_of(r0, 16), 32)
                lx_ref[r, :] = _ln(x_ref[r, :].astype(F32))

        acc = a_pass(h, 2 * L, post, **b_hooks(t, st, ln_next))
        b_finish(st, jnp.maximum(t - 3, 0))
        mem_scr[0:8, :] = acc[0:8]
        mem_scr[8:16, :] = acc[L:L + 8]
        xb_scr[0:SEG, :] = xseg(t) + acc[8:L]
        xb_scr[SEG:2 * SEG, :] = xa2 + acc[L + 8:2 * L]

    def step_single(t, layer, first=False, extra=None, ls=(0, 1)):
        st = {}
        if layer == 0:
            xa = x_ref[t * SEG:(t + 1) * SEG, :].astype(F32)
            lxa = lx_ref[t * SEG:(t + 1) * SEG, :]
        else:
            xa = x2_scr[...]
            lxa = lx2_scr[...]
        parts = [mem_scr[layer * 8:layer * 8 + 8, :], lxa]
        if extra is None:
            def post(a, p_ref, j):
                return a
        else:
            e0, en = extra
            parts.append(lx_ref[2 * SEG + e0:2 * SEG + e0 + en, :])

            def post(a, p_ref, j):
                p_ref[e0:e0 + en, j * PW:(j + 1) * PW] = a[L:L + en]
                return a[0:L]
        h = jnp.concatenate(parts, axis=0)
        if first:
            acc = a_pass(h, L, post, first=True)
        else:
            extra_mid = None
            if t == 1:
                def extra_mid():
                    cp_xr.wait()
            acc = a_pass(h, L, post, **b_hooks(t, st, extra_mid, ls))
            b_finish(st, max(t - 3, 0), ls)
        mem_scr[layer * 8:layer * 8 + 8, :] = acc[0:8]
        xb_scr[layer * SEG:(layer + 1) * SEG, :] = xa + acc[8:L]

    step_single(0, 0, first=True, extra=(0, R0))
    step_single(1, 0, extra=(R0, RN), ls=(0,))

    def body_light(t, _):
        step_double(t, True)
        return 0

    def body(t, _):
        step_double(t, False)
        return 0

    lax.fori_loop(2, 2 + NPRE, body_light, 0)
    lax.fori_loop(2 + NPRE, nseg, body, 0)
    nh = (nseg - 3) * SEG
    oc0 = pltpu.make_async_copy(o_ref.at[pl.ds(0, nh), :], o_hbm.at[pl.ds(0, nh), :], msem.at[0])
    oc0.start()
    step_single(nseg, 1)
    step_single(nseg + 1, 1, ls=(1,))
    xb, bq = b_qkv((1,))
    ob = b_attn(nseg + 2, bq, (1,))
    xo = b_out_cols(xb, ob, 0, D)
    store_out(nseg - 1, xo)
    oc1 = pltpu.make_async_copy(o_ref.at[pl.ds(nh, 3 * SEG), :], o_hbm.at[pl.ds(nh, 3 * SEG), :], msem.at[5])
    oc1.start()
    oc0.wait()
    oc1.wait()


@functools.partial(jax.jit, static_argnames=("A_seg_len",))
def pallas_interleave_layers__memory_aug_recurrent_mem_tr__sliding_local_dilated__prompt_kernel(
        A_x, A_mem0, A_Wq, A_Wk, A_Wv, A_Wo, A_seg_len, B_x, B_wqkv, B_wo):
    S = A_x.shape[1]
    x = A_x.reshape(S, D)
    mem0 = A_mem0.reshape(M, D)
    wq = A_Wq.transpose(1, 2, 0).reshape(NP * PW, D)
    wk = A_Wk.transpose(1, 2, 0).reshape(NP * PW, D)
    wv = A_Wv.transpose(1, 2, 0).reshape(NP * PW, D)
    wo = A_Wo.reshape(NP * PW, D)
    anyspec = pl.BlockSpec(memory_space=pl.ANY)
    out = pl.pallas_call(
        functools.partial(_kernel, nseg=S // SEG),
        out_shape=jax.ShapeDtypeStruct((S, D), A_x.dtype),
        in_specs=[anyspec] * 8,
        out_specs=anyspec,
        scratch_shapes=[
            pltpu.VMEM((NP, 4, PW, D), BF16),
            pltpu.VMEM((3, D, D), BF16), pltpu.VMEM((D, D), BF16),
            pltpu.VMEM((D, 3 * D), BF16), pltpu.VMEM((D, D), BF16),
            pltpu.VMEM((S, D), BF16), pltpu.VMEM((S, D), BF16), pltpu.VMEM((M, D), BF16),
            pltpu.VMEM((2 * SEG, D), F32),
            pltpu.VMEM((SEG, D), F32), pltpu.VMEM((SEG, D), F32),
            pltpu.VMEM((2 * M, D), F32),
            pltpu.VMEM((2, 16, D), F32), pltpu.VMEM((2, 16, D), F32),
            pltpu.VMEM((PROWS, NP * PW), F32), pltpu.VMEM((PROWS, NP * PW), F32), pltpu.VMEM((PROWS, NP * PW), F32),
            pltpu.VMEM((S, D), F32),
            pltpu.VMEM((NP, 3, D, PW), BF16),
            pltpu.VMEM((5, D, 128), F32),
            pltpu.SemaphoreType.DMA((NP,)),
            pltpu.SemaphoreType.DMA((8,)),
        ],
        compiler_params=pltpu.CompilerParams(vmem_limit_bytes=118 * 1024 * 1024),
    )(x, mem0, wq, wk, wv, wo, B_wqkv, B_wo)
    return out.reshape(A_x.shape)
```

```python
import functools

import jax
import jax.numpy as jnp
from jax import lax
import jax.experimental.pallas as pl
import jax.experimental.pallas.tpu as pltpu

F32 = jnp.float32
BF16 = jnp.bfloat16

SEG, M, D = 32, 8, 640
L = M + SEG
NP = 16
PW = 384
NEG = -1e9
R0 = 368
RN = 16
PROWS = 416
NPRE = (R0 + RN - SEG) // (SEG - RN) + 1
LOOK = 3
BPOS = 4
PERM0 = 8
assert RN % 16 == 0 and R0 % RN == 0 and R0 + 2 * RN <= PROWS and PROWS % RN == 0 and PROWS % SEG == 0


def _ln(x):
    m = jnp.mean(x, axis=-1, keepdims=True)
    xc = x - m
    v = jnp.mean(xc * xc, axis=-1, keepdims=True)
    return xc * lax.rsqrt(v + 1e-5)


def _dot(a, b):
    return jnp.dot(a, b, preferred_element_type=F32)


def _dot_nt(a, b):
    return lax.dot_general(a, b, (((1,), (1,)), ((), ())), preferred_element_type=F32)


def _iota(shape, dim):
    return lax.broadcasted_iota(jnp.int32, shape, dim)


def _kernel(x_hbm, mem0_hbm, wq_hbm, wk_hbm, wv_hbm, wo_hbm, bqkv_hbm, bwo_hbm, o_hbm,
            w_ref, braw_ref, bworaw_ref, bqkv_ref, bwo_ref, x_ref, o_ref, mem0_ref,
            xb_scr, x2_scr, lx2_scr, mem_scr, kprev_scr, vprev_scr,
            pq_ref, pk_ref, pv_ref, lx_ref, wn_ref, ptmp, wsem, msem, *, nseg):
    S_ROWS = nseg * SEG
    XH = 2 * SEG + R0 + SEG
    scale_a = 192 ** -0.5
    scale_b = 20 ** -0.5

    def wcopies(j):
        sl = pl.ds(j * PW, PW)
        return [pltpu.make_async_copy(hbm.at[sl, :], w_ref.at[j, i], wsem.at[j])
                for i, hbm in enumerate((wq_hbm, wk_hbm, wv_hbm, wo_hbm))]

    def start_pair(j):
        for c in wcopies(j):
            c.start()

    def wait_pair(j):
        pltpu.make_async_copy(w_ref.at[j], w_ref.at[j], wsem.at[j]).wait()

    cp_b = [pltpu.make_async_copy(bqkv_hbm.at[:, pl.ds(i * D, D)], braw_ref.at[i], msem.at[5 + i]) for i in range(3)]
    cp_bwo = pltpu.make_async_copy(bwo_hbm, bworaw_ref, msem.at[1])
    cp_xh = pltpu.make_async_copy(x_hbm.at[pl.ds(0, XH), :], x_ref.at[pl.ds(0, XH), :], msem.at[2])
    cp_mem = pltpu.make_async_copy(mem0_hbm, mem0_ref, msem.at[3])
    cp_xr = pltpu.make_async_copy(x_hbm.at[pl.ds(XH, S_ROWS - XH), :], x_ref.at[pl.ds(XH, S_ROWS - XH), :], msem.at[4])

    cp_xh.start()
    cp_mem.start()
    start_pair(0)

    xb_scr[...] = jnp.zeros_like(xb_scr)
    x2_scr[...] = jnp.zeros_like(x2_scr)
    lx2_scr[...] = jnp.zeros_like(lx2_scr)
    kprev_scr[...] = jnp.zeros_like(kprev_scr)
    vprev_scr[...] = jnp.zeros_like(vprev_scr)
    cp_xh.wait()
    cp_mem.wait()
    lx_ref[0:XH, :] = _ln(x_ref[0:XH, :].astype(F32))
    mem0 = mem0_ref[...].astype(F32)
    mem_scr[0:8, :] = mem0
    mem_scr[8:16, :] = mem0

    def perm_qkv_a(part):
        for kt in range(5):
            ptmp[kt] = braw_ref[part, kt * 128:(kt + 1) * 128, :].astype(F32).T

    def perm_qkv_b(part):
        for nt in range(5):
            for kt in range(5):
                rows = jnp.concatenate([ptmp[kt, pl.ds(4 * nt + g, 32, stride=20), :] for g in range(4)], axis=0)
                bqkv_ref[kt * 128:(kt + 1) * 128, part * D + nt * 128:part * D + (nt + 1) * 128] = rows.T.astype(BF16)

    def perm_wo():
        for ct in range(5):
            ptmp[ct] = bworaw_ref[:, ct * 128:(ct + 1) * 128].astype(F32)
        for d in range(20):
            for ct in range(5):
                bwo_ref[d * 32:(d + 1) * 32, ct * 128:(ct + 1) * 128] = ptmp[ct, pl.ds(d, 32, stride=20), :].astype(BF16)

    perm_pieces = [functools.partial(f, part) for part in range(3) for f in (perm_qkv_a, perm_qkv_b)] + [perm_wo]

    def b_qkv(ls):
        xb = xb_scr[ls[0] * SEG:(ls[-1] + 1) * SEG, :]
        hb = _ln(xb).astype(BF16)
        return xb, _dot(hb, bqkv_ref[...])

    def b_attn(t, qkv, ls):
        row = _iota((SEG, 128), 0)
        outs = []
        for i, l in enumerate(ls):
            seg = t - 1 - 2 * l
            q = qkv[i * SEG:(i + 1) * SEG, 0:D]
            k = qkv[i * SEG:(i + 1) * SEG, D:2 * D]
            v = qkv[i * SEG:(i + 1) * SEG, 2 * D:3 * D]
            kk = jnp.concatenate([kprev_scr[l], k], axis=0)
            vv = jnp.concatenate([vprev_scr[l], v], axis=0)
            kprev_scr[l] = k[16:32]
            vprev_scr[l] = v[16:32]
            logits = []
            for w in range(8):
                ks = kk[16 - 2 * w:48 - 2 * w]
                y = q[:, 0:128] * ks[:, 0:128]
                for tau in range(1, 5):
                    y = y + q[:, tau * 128:(tau + 1) * 128] * ks[:, tau * 128:(tau + 1) * 128]
                y = y + pltpu.roll(y, 64, 1)
                y = y + pltpu.roll(y, 32, 1)
                valid = (seg * SEG + row - 2 * w) >= 0
                logits.append(jnp.where(valid, y * scale_b, NEG))
            mx = logits[0]
            for w in range(1, 8):
                mx = jnp.maximum(mx, logits[w])
            es = [jnp.exp(lg - mx) for lg in logits]
            sm = es[0]
            for w in range(1, 8):
                sm = sm + es[w]
            inv = 1.0 / sm
            o_t = [None] * 5
            for w in range(8):
                p = es[w] * inv
                vs = vv[16 - 2 * w:48 - 2 * w]
                for tau in range(5):
                    term = p * vs[:, tau * 128:(tau + 1) * 128]
                    o_t[tau] = term if o_t[tau] is None else o_t[tau] + term
            outs.append(jnp.concatenate(o_t, axis=1))
        return jnp.concatenate(outs, axis=0).astype(BF16)

    def b_out_cols(xb, ob, c0, c1):
        return xb[:, c0:c1] + _dot(ob, bwo_ref[:, c0:c1])

    def t3(a):
        return a[:, 0:128], a[:, 128:256], a[:, 256:384]

    def make_att(rows):
        lo = _iota((L, 128), 1) < 64
        r = _iota((rows, 2 * L), 0)
        c = _iota((rows, 2 * L), 1)
        rl = jnp.where(r >= L, 1, 0)
        cl = jnp.where(c >= L, 1, 0)
        rr = r - rl * L
        cc = c - cl * L
        causal = (rr < M) | (rr >= cc)
        left = cl == 0
        diag = rl == cl

        def split_mid(a, swap):
            x0 = jnp.where(lo, a, 0.0)
            x1 = jnp.where(lo, 0.0, a)
            return jnp.concatenate([x1, x0] if swap else [x0, x1], axis=0).astype(BF16)

        def smax(s):
            s = jnp.where(causal, s * scale_a, NEG)
            m_lo = jnp.max(jnp.where(left, s, NEG), axis=1, keepdims=True)
            m_hi = jnp.max(jnp.where(left, NEG, s), axis=1, keepdims=True)
            e = jnp.exp(s - jnp.where(left, m_lo, m_hi))
            s_lo = jnp.sum(jnp.where(left, e, 0.0), axis=1, keepdims=True)
            s_hi = jnp.sum(jnp.where(left, 0.0, e), axis=1, keepdims=True)
            return e * jnp.where(left, 1.0 / s_lo, 1.0 / s_hi)

        if rows == L:
            zero = jnp.zeros((L, 128), F32)

            def scores(q, k):
                q0, qm, q2 = t3(q)
                k0, km, k2 = t3(k)
                r0 = jnp.concatenate([k0, zero], axis=0).astype(BF16)
                r2 = jnp.concatenate([zero, k2], axis=0).astype(BF16)
                return _dot_nt(q0, r0) + _dot_nt(q2, r2) + _dot_nt(qm, split_mid(km, False))

            def pv(p, v):
                v0, vm, v2 = t3(v)
                r0 = jnp.concatenate([v0, zero], axis=0).astype(BF16)
                r2 = jnp.concatenate([zero, v2], axis=0).astype(BF16)
                return jnp.concatenate([_dot(p, r0), _dot(p, split_mid(vm, False)), _dot(p, r2)], axis=1)
        else:
            def scores(q, k):
                q0, qm, q2 = t3(q)
                k0, km, k2 = t3(k)
                k2s = jnp.concatenate([k2[L:2 * L], k2[0:L]], axis=0)
                s0 = _dot_nt(q0, k0.astype(BF16))
                s2 = _dot_nt(q2, k2s.astype(BF16))
                mid = jnp.concatenate([_dot_nt(qm[0:L], split_mid(km[0:L], False)),
                                       _dot_nt(qm[L:2 * L], split_mid(km[L:2 * L], True))], axis=0)
                return jnp.where(diag, s0, s2) + mid

            def pv(p, v):
                v0, vm, v2 = t3(v)
                v2s = jnp.concatenate([v2[L:2 * L], v2[0:L]], axis=0)
                p0 = jnp.where(diag, p, 0.0)
                p1 = jnp.where(diag, 0.0, p)
                o0 = _dot(p0, v0.astype(BF16))
                o2 = _dot(p1, v2s.astype(BF16))
                om = jnp.concatenate([_dot(p[0:L], split_mid(vm[0:L], False)),
                                      _dot(p[L:2 * L], split_mid(vm[L:2 * L], True))], axis=0)
                return jnp.concatenate([o0, om, o2], axis=1)
        return scores, smax, pv

    def a_pass(h, rows, post, first=False, pre_hook=None, mid_hook=None, tail_x=None, tail_y=None):
        scores, smax, pv = make_att(rows)
        started = [1]

        def wait(j):
            if first:
                wait_pair(j)
                for js in range(started[0], min(NP, j + 1 + LOOK)):
                    start_pair(js)
                    started[0] = js + 1
                if j == BPOS:
                    for c in cp_b + [cp_bwo]:
                        c.start()
                if j == PERM0 + 1:
                    for c in cp_b + [cp_bwo]:
                        c.wait()
                if j == NP - 1:
                    cp_xr.start()

        def proj(i, p_ref, j):
            if first:
                return post(_dot_nt(h, w_ref[j, i]), p_ref, j)
            return post(_dot(h, wn_ref[j, i]), p_ref, j)

        def outproj(o, j):
            return _dot(o, w_ref[j, 3])

        wait(0)
        q = proj(0, pq_ref, 0)
        k = proj(1, pk_ref, 0)
        v = proj(2, pv_ref, 0)
        if pre_hook is not None:
            pre_hook()
        acc = None
        o_def = None
        for j in range(NP):
            s = scores(q, k)
            if j < NP - 1:
                wait(j + 1)
                qn = proj(0, pq_ref, j + 1)
                kn = proj(1, pk_ref, j + 1)
            else:
                acc = acc + outproj(o_def, j - 1)
                if tail_x is not None:
                    tail_x()
            p = smax(s)
            if j == 8 and mid_hook is not None:
                mid_hook()
            o = pv(p, v)
            if j < NP - 1:
                vn = proj(2, pv_ref, j + 1)
            elif tail_y is not None:
                tail_y()
            if j == NP - 2:
                o_def = o
            else:
                contrib = outproj(o, j)
                acc = contrib if acc is None else acc + contrib
            if first and PERM0 <= j < PERM0 + len(perm_pieces):
                perm_pieces[j - PERM0]()
            if first:
                for i in range(3):
                    wn_ref[j, i] = w_ref[j, i].T
            if j < NP - 1:
                q, k, v = qn, kn, vn
        return acc

    def xseg(s):
        return x_ref[pl.ds(pl.multiple_of(s * SEG, SEG), SEG), :].astype(F32)

    def lxrows(r0, n):
        return lx_ref[pl.ds(pl.multiple_of(r0, 8), n), :]

    def store_out(s, val):
        o_ref[pl.ds(pl.multiple_of(s * SEG, SEG), SEG), :] = val.astype(o_ref.dtype)

    def b_hooks(t, st, extra_mid=None, ls=(0, 1)):
        def pre():
            st['xb'], st['bq'] = b_qkv(ls)

        def mid():
            st['ob'] = b_attn(t, st['bq'], ls)
            if extra_mid is not None:
                extra_mid()

        def tx():
            st['xo0'] = b_out_cols(st['xb'], st['ob'], 0, 384)

        def ty():
            st['xo1'] = b_out_cols(st['xb'], st['ob'], 384, 640)
        return dict(pre_hook=pre, mid_hook=mid, tail_x=tx, tail_y=ty)

    def b_finish(st, so, ls=(0, 1)):
        xo = jnp.concatenate([st['xo0'], st['xo1']], axis=1)
        if 0 in ls:
            x2_scr[...] = xo[0:SEG]
            lx2_scr[...] = _ln(xo[0:SEG])
        if 1 in ls:
            store_out(so, xo[(len(ls) - 1) * SEG:len(ls) * SEG])

    def step_double(t, light):
        st = {}
        xa2 = x2_scr[...]
        mem12 = mem_scr[...]
        lx2 = lx2_scr[...]
        if light:
            rnew = R0 + RN + RN * (t - 2)
            pnew = pl.multiple_of(lax.rem(rnew, PROWS), 8)
            pcur = pl.multiple_of(lax.rem(SEG * (t - 2), PROWS), 8)
            h = jnp.concatenate([mem12, lx2, lxrows(rnew + 2 * SEG, RN)], axis=0).astype(BF16)
            nxt = (rnew + RN + 2 * SEG, RN)

            def post(a, p_ref, j):
                cols = slice(j * PW, (j + 1) * PW)
                p_ref[pl.ds(pnew, RN), cols] = a[48:48 + RN]
                return jnp.concatenate([a[0:8], p_ref[pl.ds(pcur, SEG), cols], a[8:48]], axis=0)
        else:
            h = jnp.concatenate([mem12.astype(BF16), lxrows(t * SEG, SEG).astype(BF16), lx2.astype(BF16)], axis=0)

            def post(a, p_ref, j):
                return jnp.concatenate([a[0:8], a[16:48], a[8:16], a[48:80]], axis=0)
            nxt = (jnp.minimum(t + 1, nseg - 1) * SEG, SEG)

        def ln_next():
            r = pl.ds(pl.multiple_of(nxt[0], 16), nxt[1])
            lx_ref[r, :] = _ln(x_ref[r, :].astype(F32))

        acc = a_pass(h, 2 * L, post, **b_hooks(t, st, ln_next))
        b_finish(st, jnp.maximum(t - 3, 0))
        mem_scr[0:8, :] = acc[0:8]
        mem_scr[8:16, :] = acc[L:L + 8]
        xb_scr[0:SEG, :] = xseg(t) + acc[8:L]
        xb_scr[SEG:2 * SEG, :] = xa2 + acc[L + 8:2 * L]

    def step_single(t, layer, first=False, extra=None, ls=(0, 1)):
        st = {}
        if layer == 0:
            xa = x_ref[t * SEG:(t + 1) * SEG, :].astype(F32)
            lxa = lx_ref[t * SEG:(t + 1) * SEG, :]
        else:
            xa = x2_scr[...]
            lxa = lx2_scr[...]
        parts = [mem_scr[layer * 8:layer * 8 + 8, :], lxa]
        if extra is None:
            def post(a, p_ref, j):
                return a
        else:
            e0, en = extra
            parts.append(lx_ref[2 * SEG + e0:2 * SEG + e0 + en, :])

            def post(a, p_ref, j):
                p_ref[e0:e0 + en, j * PW:(j + 1) * PW] = a[L:L + en]
                return a[0:L]
        h = jnp.concatenate(parts, axis=0)
        if first:
            acc = a_pass(h, L, post, first=True)
        else:
            extra_mid = None
            if t == 1:
                def extra_mid():
                    cp_xr.wait()
            acc = a_pass(h, L, post, **b_hooks(t, st, extra_mid, ls))
            b_finish(st, max(t - 3, 0), ls)
        mem_scr[layer * 8:layer * 8 + 8, :] = acc[0:8]
        xb_scr[layer * SEG:(layer + 1) * SEG, :] = xa + acc[8:L]

    step_single(0, 0, first=True, extra=(0, R0))
    step_single(1, 0, extra=(R0, RN), ls=(0,))

    def body_light(t, _):
        step_double(t, True)
        return 0

    def body(t, _):
        step_double(t, False)
        return 0

    lax.fori_loop(2, 2 + NPRE, body_light, 0)
    lax.fori_loop(2 + NPRE, nseg, body, 0)
    nh = (nseg - 3) * SEG
    oc0 = pltpu.make_async_copy(o_ref.at[pl.ds(0, nh), :], o_hbm.at[pl.ds(0, nh), :], msem.at[0])
    oc0.start()
    step_single(nseg, 1)
    step_single(nseg + 1, 1, ls=(1,))
    xb, bq = b_qkv((1,))
    ob = b_attn(nseg + 2, bq, (1,))
    xo = b_out_cols(xb, ob, 0, D)
    store_out(nseg - 1, xo)
    oc1 = pltpu.make_async_copy(o_ref.at[pl.ds(nh, 3 * SEG), :], o_hbm.at[pl.ds(nh, 3 * SEG), :], msem.at[5])
    oc1.start()
    oc0.wait()
    oc1.wait()


@functools.partial(jax.jit, static_argnames=("A_seg_len",))
def pallas_interleave_layers__memory_aug_recurrent_mem_tr__sliding_local_dilated__prompt_kernel(
        A_x, A_mem0, A_Wq, A_Wk, A_Wv, A_Wo, A_seg_len, B_x, B_wqkv, B_wo):
    S = A_x.shape[1]
    assert A_x.shape == (1, S, D) and S % SEG == 0 and A_seg_len == SEG and S // SEG >= 3 + NPRE
    assert A_mem0.shape == (1, M, D) and A_Wq.shape == (D, 2 * NP, PW // 2) and B_wqkv.shape == (D, 3 * D)
    x = A_x.reshape(S, D)
    mem0 = A_mem0.reshape(M, D)
    wq = A_Wq.transpose(1, 2, 0).reshape(NP * PW, D)
    wk = A_Wk.transpose(1, 2, 0).reshape(NP * PW, D)
    wv = A_Wv.transpose(1, 2, 0).reshape(NP * PW, D)
    wo = A_Wo.reshape(NP * PW, D)
    anyspec = pl.BlockSpec(memory_space=pl.ANY)
    out = pl.pallas_call(
        functools.partial(_kernel, nseg=S // SEG),
        out_shape=jax.ShapeDtypeStruct((S, D), A_x.dtype),
        in_specs=[anyspec] * 8,
        out_specs=anyspec,
        scratch_shapes=[
            pltpu.VMEM((NP, 4, PW, D), BF16),
            pltpu.VMEM((3, D, D), BF16), pltpu.VMEM((D, D), BF16),
            pltpu.VMEM((D, 3 * D), BF16), pltpu.VMEM((D, D), BF16),
            pltpu.VMEM((S, D), BF16), pltpu.VMEM((S, D), BF16), pltpu.VMEM((M, D), BF16),
            pltpu.VMEM((2 * SEG, D), F32),
            pltpu.VMEM((SEG, D), F32), pltpu.VMEM((SEG, D), F32),
            pltpu.VMEM((2 * M, D), F32),
            pltpu.VMEM((2, 16, D), F32), pltpu.VMEM((2, 16, D), F32),
            pltpu.VMEM((PROWS, NP * PW), F32), pltpu.VMEM((PROWS, NP * PW), F32), pltpu.VMEM((PROWS, NP * PW), F32),
            pltpu.VMEM((S, D), F32),
            pltpu.VMEM((NP, 3, D, PW), BF16),
            pltpu.VMEM((5, D, 128), F32),
            pltpu.SemaphoreType.DMA((NP,)),
            pltpu.SemaphoreType.DMA((8,)),
        ],
        compiler_params=pltpu.CompilerParams(vmem_limit_bytes=118 * 1024 * 1024),
    )(x, mem0, wq, wk, wv, wo, B_wqkv, B_wo)
    return out.reshape(A_x.shape)
```

```python
import functools

import jax
import jax.numpy as jnp
from jax import lax
import jax.experimental.pallas as pl
import jax.experimental.pallas.tpu as pltpu

F32 = jnp.float32
BF16 = jnp.bfloat16

SEG, M, D = 32, 8, 640
L = M + SEG
NP = 16
PW = 384
NEG = -1e9
R0 = 368
RN = 16
PROWS = 416
NPRE = (R0 + RN - SEG) // (SEG - RN) + 1
LOOK = 4
BPOS = 4
PERM0 = 8
assert RN % 16 == 0 and R0 % RN == 0 and R0 + 2 * RN <= PROWS and PROWS % RN == 0 and PROWS % SEG == 0


def _ln(x):
    m = jnp.mean(x, axis=-1, keepdims=True)
    xc = x - m
    v = jnp.mean(xc * xc, axis=-1, keepdims=True)
    return xc * lax.rsqrt(v + 1e-5)


def _dot(a, b):
    return jnp.dot(a, b, preferred_element_type=F32)


def _dot_nt(a, b):
    return lax.dot_general(a, b, (((1,), (1,)), ((), ())), preferred_element_type=F32)


def _iota(shape, dim):
    return lax.broadcasted_iota(jnp.int32, shape, dim)


def _kernel(x_hbm, mem0_hbm, wq_hbm, wk_hbm, wv_hbm, wo_hbm, bqkv_hbm, bwo_hbm, o_hbm,
            w_ref, braw_ref, bworaw_ref, bqkv_ref, bwo_ref, x_ref, o_ref, mem0_ref,
            xb_scr, x2_scr, lx2_scr, mem_scr, kprev_scr, vprev_scr,
            pq_ref, pk_ref, pv_ref, lx_ref, wn_ref, ptmp, wsem, msem, *, nseg):
    S_ROWS = nseg * SEG
    XH = 2 * SEG + R0 + SEG
    scale_a = 192 ** -0.5
    scale_b = 20 ** -0.5

    def wcopy(hbm, jj, slab, i):
        return pltpu.make_async_copy(hbm.at[pl.ds(jj * PW, PW), :], w_ref.at[slab, i], wsem.at[slab if i < 3 else jj + 1])

    def start_pair(j):
        for i, hbm in enumerate((wq_hbm, wk_hbm, wv_hbm)):
            wcopy(hbm, j, j, i).start()
        if j > 0:
            wcopy(wo_hbm, j - 1, j, 3).start()
        if j == NP - 1:
            wcopy(wo_hbm, j, 0, 3).start()

    def wait_pair(j):
        slab = w_ref.at[j] if j else w_ref.at[0, pl.ds(0, 3)]
        pltpu.make_async_copy(slab, slab, wsem.at[j]).wait()
        if j == NP - 1:
            wcopy(wo_hbm, j, 0, 3).wait()

    cp_b = [pltpu.make_async_copy(bqkv_hbm.at[:, pl.ds(i * D, D)], braw_ref.at[i], msem.at[5 + i]) for i in range(3)]
    cp_bwo = pltpu.make_async_copy(bwo_hbm, bworaw_ref, msem.at[1])
    cp_xh = pltpu.make_async_copy(x_hbm.at[pl.ds(0, XH), :], x_ref.at[pl.ds(0, XH), :], msem.at[2])
    cp_mem = pltpu.make_async_copy(mem0_hbm, mem0_ref, msem.at[3])
    cp_xr = pltpu.make_async_copy(x_hbm.at[pl.ds(XH, S_ROWS - XH), :], x_ref.at[pl.ds(XH, S_ROWS - XH), :], msem.at[4])

    cp_xh.start()
    cp_mem.start()
    start_pair(0)

    xb_scr[...] = jnp.zeros_like(xb_scr)
    x2_scr[...] = jnp.zeros_like(x2_scr)
    lx2_scr[...] = jnp.zeros_like(lx2_scr)
    kprev_scr[...] = jnp.zeros_like(kprev_scr)
    vprev_scr[...] = jnp.zeros_like(vprev_scr)
    cp_xh.wait()
    cp_mem.wait()
    lx_ref[0:XH, :] = _ln(x_ref[0:XH, :].astype(F32))
    mem0 = mem0_ref[...].astype(F32)
    mem_scr[0:8, :] = mem0
    mem_scr[8:16, :] = mem0

    def perm_qkv_a(part):
        for kt in range(5):
            ptmp[kt] = braw_ref[part, kt * 128:(kt + 1) * 128, :].astype(F32).T

    def perm_qkv_b(part):
        for nt in range(5):
            for kt in range(5):
                rows = jnp.concatenate([ptmp[kt, pl.ds(4 * nt + g, 32, stride=20), :] for g in range(4)], axis=0)
                bqkv_ref[kt * 128:(kt + 1) * 128, part * D + nt * 128:part * D + (nt + 1) * 128] = rows.T.astype(BF16)

    def perm_wo():
        for ct in range(5):
            ptmp[ct] = bworaw_ref[:, ct * 128:(ct + 1) * 128].astype(F32)
        for d in range(20):
            for ct in range(5):
                bwo_ref[d * 32:(d + 1) * 32, ct * 128:(ct + 1) * 128] = ptmp[ct, pl.ds(d, 32, stride=20), :].astype(BF16)

    perm_pieces = [functools.partial(f, part) for part in range(3) for f in (perm_qkv_a, perm_qkv_b)] + [perm_wo]

    def b_qkv(ls):
        xb = xb_scr[ls[0] * SEG:(ls[-1] + 1) * SEG, :]
        hb = _ln(xb).astype(BF16)
        return xb, _dot(hb, bqkv_ref[...])

    def b_attn(t, qkv, ls):
        row = _iota((SEG, 128), 0)
        outs = []
        for i, l in enumerate(ls):
            seg = t - 1 - 2 * l
            q = qkv[i * SEG:(i + 1) * SEG, 0:D]
            k = qkv[i * SEG:(i + 1) * SEG, D:2 * D]
            v = qkv[i * SEG:(i + 1) * SEG, 2 * D:3 * D]
            kk = jnp.concatenate([kprev_scr[l], k], axis=0)
            vv = jnp.concatenate([vprev_scr[l], v], axis=0)
            kprev_scr[l] = k[16:32]
            vprev_scr[l] = v[16:32]
            logits = []
            for w in range(8):
                ks = kk[16 - 2 * w:48 - 2 * w]
                y = q[:, 0:128] * ks[:, 0:128]
                for tau in range(1, 5):
                    y = y + q[:, tau * 128:(tau + 1) * 128] * ks[:, tau * 128:(tau + 1) * 128]
                y = y + pltpu.roll(y, 64, 1)
                y = y + pltpu.roll(y, 32, 1)
                valid = (seg * SEG + row - 2 * w) >= 0
                logits.append(jnp.where(valid, y * scale_b, NEG))
            mx = logits[0]
            for w in range(1, 8):
                mx = jnp.maximum(mx, logits[w])
            es = [jnp.exp(lg - mx) for lg in logits]
            sm = es[0]
            for w in range(1, 8):
                sm = sm + es[w]
            inv = 1.0 / sm
            o_t = [None] * 5
            for w in range(8):
                p = es[w] * inv
                vs = vv[16 - 2 * w:48 - 2 * w]
                for tau in range(5):
                    term = p * vs[:, tau * 128:(tau + 1) * 128]
                    o_t[tau] = term if o_t[tau] is None else o_t[tau] + term
            outs.append(jnp.concatenate(o_t, axis=1))
        return jnp.concatenate(outs, axis=0).astype(BF16)

    def b_out_cols(xb, ob, c0, c1):
        return xb[:, c0:c1] + _dot(ob, bwo_ref[:, c0:c1])

    def t3(a):
        return a[:, 0:128], a[:, 128:256], a[:, 256:384]

    def make_att(rows):
        lo = _iota((L, 128), 1) < 64
        r = _iota((rows, 2 * L), 0)
        c = _iota((rows, 2 * L), 1)
        rl = jnp.where(r >= L, 1, 0)
        cl = jnp.where(c >= L, 1, 0)
        rr = r - rl * L
        cc = c - cl * L
        causal = (rr < M) | (rr >= cc)
        left = cl == 0
        diag = rl == cl

        def split_mid(a, swap):
            x0 = jnp.where(lo, a, 0.0)
            x1 = jnp.where(lo, 0.0, a)
            return jnp.concatenate([x1, x0] if swap else [x0, x1], axis=0).astype(BF16)

        def smax(s):
            s = jnp.where(causal, s * scale_a, NEG)
            m_lo = jnp.max(jnp.where(left, s, NEG), axis=1, keepdims=True)
            m_hi = jnp.max(jnp.where(left, NEG, s), axis=1, keepdims=True)
            e = jnp.exp(s - jnp.where(left, m_lo, m_hi))
            s_lo = jnp.sum(jnp.where(left, e, 0.0), axis=1, keepdims=True)
            s_hi = jnp.sum(jnp.where(left, 0.0, e), axis=1, keepdims=True)
            return e * jnp.where(left, 1.0 / s_lo, 1.0 / s_hi)

        if rows == L:
            zero = jnp.zeros((L, 128), F32)

            def scores(q, k):
                q0, qm, q2 = t3(q)
                k0, km, k2 = t3(k)
                r0 = jnp.concatenate([k0, zero], axis=0).astype(BF16)
                r2 = jnp.concatenate([zero, k2], axis=0).astype(BF16)
                return _dot_nt(q0, r0) + _dot_nt(q2, r2) + _dot_nt(qm, split_mid(km, False))

            def pv(p, v):
                v0, vm, v2 = t3(v)
                r0 = jnp.concatenate([v0, zero], axis=0).astype(BF16)
                r2 = jnp.concatenate([zero, v2], axis=0).astype(BF16)
                return jnp.concatenate([_dot(p, r0), _dot(p, split_mid(vm, False)), _dot(p, r2)], axis=1)
        else:
            def scores(q, k):
                q0, qm, q2 = t3(q)
                k0, km, k2 = t3(k)
                k2s = jnp.concatenate([k2[L:2 * L], k2[0:L]], axis=0)
                s0 = _dot_nt(q0, k0.astype(BF16))
                s2 = _dot_nt(q2, k2s.astype(BF16))
                mid = jnp.concatenate([_dot_nt(qm[0:L], split_mid(km[0:L], False)),
                                       _dot_nt(qm[L:2 * L], split_mid(km[L:2 * L], True))], axis=0)
                return jnp.where(diag, s0, s2) + mid

            def pv(p, v):
                v0, vm, v2 = t3(v)
                v2s = jnp.concatenate([v2[L:2 * L], v2[0:L]], axis=0)
                p0 = jnp.where(diag, p, 0.0)
                p1 = jnp.where(diag, 0.0, p)
                o0 = _dot(p0, v0.astype(BF16))
                o2 = _dot(p1, v2s.astype(BF16))
                om = jnp.concatenate([_dot(p[0:L], split_mid(vm[0:L], False)),
                                      _dot(p[L:2 * L], split_mid(vm[L:2 * L], True))], axis=0)
                return jnp.concatenate([o0, om, o2], axis=1)
        return scores, smax, pv

    def a_pass(h, rows, post, first=False, pre_hook=None, mid_hook=None, tail_x=None, tail_y=None):
        scores, smax, pv = make_att(rows)
        started = [1]

        def wait(j):
            if first:
                wait_pair(j)
                for js in range(started[0], min(NP, j + 1 + LOOK)):
                    start_pair(js)
                    started[0] = js + 1
                if j == BPOS:
                    for c in cp_b + [cp_bwo]:
                        c.start()
                if j == PERM0 + 1:
                    for c in cp_b + [cp_bwo]:
                        c.wait()
                if j == NP - 1:
                    cp_xr.start()

        def proj(i, p_ref, j):
            if first:
                return post(_dot_nt(h, w_ref[j, i]), p_ref, j)
            return post(_dot(h, wn_ref[j, i]), p_ref, j)

        def outproj(o, j):
            return _dot(o, w_ref[(j + 1) % NP, 3])

        wait(0)
        q = proj(0, pq_ref, 0)
        k = proj(1, pk_ref, 0)
        v = proj(2, pv_ref, 0)
        if pre_hook is not None:
            pre_hook()
        acc = None
        o_def = None
        for j in range(NP):
            s = scores(q, k)
            if j < NP - 1:
                wait(j + 1)
                qn = proj(0, pq_ref, j + 1)
                kn = proj(1, pk_ref, j + 1)
            else:
                acc = acc + outproj(o_def, j - 1)
                if tail_x is not None:
                    tail_x()
            p = smax(s)
            if j == 8 and mid_hook is not None:
                mid_hook()
            o = pv(p, v)
            if j < NP - 1:
                vn = proj(2, pv_ref, j + 1)
            elif tail_y is not None:
                tail_y()
            if j == NP - 2:
                o_def = o
            else:
                contrib = outproj(o, j)
                acc = contrib if acc is None else acc + contrib
            if first and PERM0 <= j < PERM0 + len(perm_pieces):
                perm_pieces[j - PERM0]()
            if first:
                for i in range(3):
                    wn_ref[j, i] = w_ref[j, i].T
            if j < NP - 1:
                q, k, v = qn, kn, vn
        return acc

    def xseg(s):
        return x_ref[pl.ds(pl.multiple_of(s * SEG, SEG), SEG), :].astype(F32)

    def lxrows(r0, n):
        return lx_ref[pl.ds(pl.multiple_of(r0, 8), n), :]

    def store_out(s, val):
        o_ref[pl.ds(pl.multiple_of(s * SEG, SEG), SEG), :] = val.astype(o_ref.dtype)

    def b_hooks(t, st, extra_mid=None, ls=(0, 1)):
        def pre():
            st['xb'], st['bq'] = b_qkv(ls)

        def mid():
            st['ob'] = b_attn(t, st['bq'], ls)
            if extra_mid is not None:
                extra_mid()

        def tx():
            st['xo0'] = b_out_cols(st['xb'], st['ob'], 0, 384)

        def ty():
            st['xo1'] = b_out_cols(st['xb'], st['ob'], 384, 640)
        return dict(pre_hook=pre, mid_hook=mid, tail_x=tx, tail_y=ty)

    def b_finish(st, so, ls=(0, 1)):
        xo = jnp.concatenate([st['xo0'], st['xo1']], axis=1)
        if 0 in ls:
            x2_scr[...] = xo[0:SEG]
            lx2_scr[...] = _ln(xo[0:SEG])
        if 1 in ls:
            store_out(so, xo[(len(ls) - 1) * SEG:len(ls) * SEG])

    def step_double(t, light):
        st = {}
        xa2 = x2_scr[...]
        mem12 = mem_scr[...]
        lx2 = lx2_scr[...]
        if light:
            rnew = R0 + RN + RN * (t - 2)
            pnew = pl.multiple_of(lax.rem(rnew, PROWS), 8)
            pcur = pl.multiple_of(lax.rem(SEG * (t - 2), PROWS), 8)
            h = jnp.concatenate([mem12, lx2, lxrows(rnew + 2 * SEG, RN)], axis=0).astype(BF16)
            nxt = (rnew + RN + 2 * SEG, RN)

            def post(a, p_ref, j):
                cols = slice(j * PW, (j + 1) * PW)
                p_ref[pl.ds(pnew, RN), cols] = a[48:48 + RN]
                return jnp.concatenate([a[0:8], p_ref[pl.ds(pcur, SEG), cols], a[8:48]], axis=0)
        else:
            h = jnp.concatenate([mem12.astype(BF16), lxrows(t * SEG, SEG).astype(BF16), lx2.astype(BF16)], axis=0)

            def post(a, p_ref, j):
                return jnp.concatenate([a[0:8], a[16:48], a[8:16], a[48:80]], axis=0)
            nxt = (jnp.minimum(t + 1, nseg - 1) * SEG, SEG)

        def ln_next():
            r = pl.ds(pl.multiple_of(nxt[0], 16), nxt[1])
            lx_ref[r, :] = _ln(x_ref[r, :].astype(F32))

        acc = a_pass(h, 2 * L, post, **b_hooks(t, st, ln_next))
        b_finish(st, jnp.maximum(t - 3, 0))
        mem_scr[0:8, :] = acc[0:8]
        mem_scr[8:16, :] = acc[L:L + 8]
        xb_scr[0:SEG, :] = xseg(t) + acc[8:L]
        xb_scr[SEG:2 * SEG, :] = xa2 + acc[L + 8:2 * L]

    def step_single(t, layer, first=False, extra=None, ls=(0, 1)):
        st = {}
        if layer == 0:
            xa = x_ref[t * SEG:(t + 1) * SEG, :].astype(F32)
            lxa = lx_ref[t * SEG:(t + 1) * SEG, :]
        else:
            xa = x2_scr[...]
            lxa = lx2_scr[...]
        parts = [mem_scr[layer * 8:layer * 8 + 8, :], lxa]
        if extra is None:
            def post(a, p_ref, j):
                return a
        else:
            e0, en = extra
            parts.append(lx_ref[2 * SEG + e0:2 * SEG + e0 + en, :])

            def post(a, p_ref, j):
                p_ref[e0:e0 + en, j * PW:(j + 1) * PW] = a[L:L + en]
                return a[0:L]
        h = jnp.concatenate(parts, axis=0)
        if first:
            acc = a_pass(h, L, post, first=True)
        else:
            extra_mid = None
            if t == 1:
                def extra_mid():
                    cp_xr.wait()
            acc = a_pass(h, L, post, **b_hooks(t, st, extra_mid, ls))
            b_finish(st, max(t - 3, 0), ls)
        mem_scr[layer * 8:layer * 8 + 8, :] = acc[0:8]
        xb_scr[layer * SEG:(layer + 1) * SEG, :] = xa + acc[8:L]

    step_single(0, 0, first=True, extra=(0, R0))
    step_single(1, 0, extra=(R0, RN), ls=(0,))

    def body_light(t, _):
        step_double(t, True)
        return 0

    def body(t, _):
        step_double(t, False)
        return 0

    lax.fori_loop(2, 2 + NPRE, body_light, 0)
    lax.fori_loop(2 + NPRE, nseg, body, 0)
    nh = (nseg - 3) * SEG
    oc0 = pltpu.make_async_copy(o_ref.at[pl.ds(0, nh), :], o_hbm.at[pl.ds(0, nh), :], msem.at[0])
    oc0.start()
    step_single(nseg, 1)
    step_single(nseg + 1, 1, ls=(1,))
    xb, bq = b_qkv((1,))
    ob = b_attn(nseg + 2, bq, (1,))
    xo = b_out_cols(xb, ob, 0, D)
    store_out(nseg - 1, xo)
    oc1 = pltpu.make_async_copy(o_ref.at[pl.ds(nh, 3 * SEG), :], o_hbm.at[pl.ds(nh, 3 * SEG), :], msem.at[5])
    oc1.start()
    oc0.wait()
    oc1.wait()


@functools.partial(jax.jit, static_argnames=("A_seg_len",))
def pallas_interleave_layers__memory_aug_recurrent_mem_tr__sliding_local_dilated__prompt_kernel(
        A_x, A_mem0, A_Wq, A_Wk, A_Wv, A_Wo, A_seg_len, B_x, B_wqkv, B_wo):
    S = A_x.shape[1]
    assert A_x.shape == (1, S, D) and S % SEG == 0 and A_seg_len == SEG and S // SEG >= 3 + NPRE
    assert A_mem0.shape == (1, M, D) and A_Wq.shape == (D, 2 * NP, PW // 2) and B_wqkv.shape == (D, 3 * D)
    x = A_x.reshape(S, D)
    mem0 = A_mem0.reshape(M, D)
    wq = A_Wq.transpose(1, 2, 0).reshape(NP * PW, D)
    wk = A_Wk.transpose(1, 2, 0).reshape(NP * PW, D)
    wv = A_Wv.transpose(1, 2, 0).reshape(NP * PW, D)
    wo = A_Wo.reshape(NP * PW, D)
    anyspec = pl.BlockSpec(memory_space=pl.ANY)
    out = pl.pallas_call(
        functools.partial(_kernel, nseg=S // SEG),
        out_shape=jax.ShapeDtypeStruct((S, D), A_x.dtype),
        in_specs=[anyspec] * 8,
        out_specs=anyspec,
        scratch_shapes=[
            pltpu.VMEM((NP, 4, PW, D), BF16),
            pltpu.VMEM((3, D, D), BF16), pltpu.VMEM((D, D), BF16),
            pltpu.VMEM((D, 3 * D), BF16), pltpu.VMEM((D, D), BF16),
            pltpu.VMEM((S, D), BF16), pltpu.VMEM((S, D), BF16), pltpu.VMEM((M, D), BF16),
            pltpu.VMEM((2 * SEG, D), F32),
            pltpu.VMEM((SEG, D), F32), pltpu.VMEM((SEG, D), F32),
            pltpu.VMEM((2 * M, D), F32),
            pltpu.VMEM((2, 16, D), F32), pltpu.VMEM((2, 16, D), F32),
            pltpu.VMEM((PROWS, NP * PW), F32), pltpu.VMEM((PROWS, NP * PW), F32), pltpu.VMEM((PROWS, NP * PW), F32),
            pltpu.VMEM((S, D), F32),
            pltpu.VMEM((NP, 3, D, PW), BF16),
            pltpu.VMEM((5, D, 128), F32),
            pltpu.SemaphoreType.DMA((NP + 1,)),
            pltpu.SemaphoreType.DMA((8,)),
        ],
        compiler_params=pltpu.CompilerParams(vmem_limit_bytes=118 * 1024 * 1024),
    )(x, mem0, wq, wk, wv, wo, B_wqkv, B_wo)
    return out.reshape(A_x.shape)
```
